```python
import jax
import jax.numpy as jnp

def _softmax(x, axis=-1):
    return jax.nn.softmax(x, axis=axis)
def _gelu(x):
    return jax.nn.gelu(x, approximate=True)
def _silu(x):
    return jax.nn.silu(x)
def _sigmoid(x):
    return jax.nn.sigmoid(x)
def _layernorm(x, axis=-1, eps=1e-5):
    m = jnp.mean(x, axis=axis, keepdims=True)
    v = jnp.var(x, axis=axis, keepdims=True)
    return (x - m) / jnp.sqrt(v + eps)
def _scatter_add(tgt, idx, src, axis=0):
    return tgt.at[idx].add(src)
def _segment_sum(src, seg, n):
    return jax.ops.segment_sum(src, seg, n)
class _Rng:
    def __init__(self, key):
        self._k = key
    def _next(self):
        self._k, sub = jax.random.split(self._k)
        return sub
    def normal(self, shape):
        return jax.random.normal(self._next(), shape, dtype=jnp.bfloat16)
    def randint(self, lo, hi, shape):
        return jax.random.randint(self._next(), shape, lo, hi, dtype=jnp.int32)
    def uniform(self, shape, lo=0.0, hi=1.0):
        return jax.random.uniform(self._next(), shape, jnp.bfloat16, lo, hi)
    def permutation(self, n):
        return jax.random.permutation(self._next(), n)


kernel_name = 'recurrent_scan__sliding_local_dilated__geglu_ffn__prompt'

def setup_inputs():
    _rng = _Rng(jax.random.key(int.from_bytes(__import__("os").urandom(4), "little")))
    _w = (lambda a: (lambda t: t.astype(jnp.bfloat16) if jnp.issubdtype(t.dtype, jnp.floating) else t)(jnp.asarray(a)))
    def _A_setup():
        B, S, D = 1, 2048, 1024
        return {
            "x": _w((lambda *s: _rng.normal(s) * 0.05)(B, S, D)),
            "wqkv": _w((lambda *s: _rng.normal(s) * 0.05)(D, 3 * D)),
            "wo": _w((lambda *s: _rng.normal(s) * 0.05)(D, D)),
        }
    _A_in = _A_setup()

    def _B_setup():
        B, S, D, F = 1, 2048, 1024, 3584
        return {
            "x": _w((lambda *s: _rng.normal(s) * 0.05)(B, S, D)),
            "w_gate": _w((lambda *s: _rng.normal(s) * 0.05)(D, F)),
            "w_up": _w((lambda *s: _rng.normal(s) * 0.05)(D, F)),
            "w_down": _w((lambda *s: _rng.normal(s) * 0.05)(F, D)),
        }
    _B_in = _B_setup()

    return {
        "A_x": _A_in["x"],
        "A_wqkv": _A_in["wqkv"],
        "A_wo": _A_in["wo"],
        "B_x": _B_in["x"],
        "B_w_gate": _B_in["w_gate"],
        "B_w_up": _B_in["w_up"],
        "B_w_down": _B_in["w_down"],
    }

def reference(A_x, A_wqkv, A_wo, B_x, B_w_gate, B_w_up, B_w_down):
    def _A_ref(x, wqkv, wo):
        B, S, D = x.shape
        H = 32; Dh = D // H
        W, dil = 8, 2
        qkv = (lambda x, *d: x.transpose(*d))((x @ wqkv).reshape(B, S, 3, H, Dh), 2, 0, 3, 1, 4)
        q, k, v = qkv[0], qkv[1], qkv[2]
        scale = Dh ** -0.5
        pos = jnp.arange(S)
        off = jnp.arange(W) * dil
        idx = pos[:, None] - off[None, :]
        mask = idx >= 0
        idx_c = jnp.where(mask, idx, 0).reshape(-1)
        kg = k[:, :, idx_c, :].reshape(B, H, S, W, Dh)
        vg = v[:, :, idx_c, :].reshape(B, H, S, W, Dh)
        logits = jnp.einsum("bhsd,bhswd->bhsw", q, kg) * scale
        logits = jnp.where(mask[None, None, :, :], logits, -1e9)
        attn = _softmax(logits, axis=-1)
        o = jnp.einsum("bhsw,bhswd->bhsd", attn, vg)
        return (lambda x, *d: x.transpose(*d))(o, 0, 2, 1, 3).reshape(B, S, D) @ wo

    def _B_ref(x, w_gate, w_up, w_down):
        return (_gelu(x @ w_gate) * (x @ w_up)) @ w_down

    x = A_x
    xn = _layernorm(x, axis=-1)
    s = _A_ref(xn, A_wqkv, A_wo)
    g = _silu(_B_ref(xn, B_w_gate, B_w_up, B_w_down))
    return x + s * g
```

```python
import functools
import numpy as np
import jax
import jax.numpy as jnp
from jax import lax
from jax.experimental import pallas as pl
from jax.experimental.pallas import tpu as pltpu

S, D, F = 2048, 1024, 3584
DH, WIN, DIL = 32, 8, 2
BM = 256
HM = BM // 2
NB = S // BM
FC = 256
HF = FC // 2
NC = F // FC
HD = D // 2
HALO = 16
F32, BF16 = jnp.float32, jnp.bfloat16
ORDER = (1, 4, 2, 3, 5, 6, 0)


def _lhs_ops(a11, a12, a21, a22):
    ops = (a11 + a22, a21 + a22, a11, a22, a11 + a12, a21 - a11, a12 - a22)
    return [o.astype(BF16) for o in ops]


def _rhs_ops(b11, b12, b21, b22):
    f11, f12, f21, f22 = (b.astype(F32) for b in (b11, b12, b21, b22))
    r = lambda t: t.astype(BF16)
    return [r(f11 + f22), r(b11), r(f12 - f22), r(f21 - f11), r(b22), r(f11 + f12), r(f21 + f22)]


def _block_matmul(lhs, rhs, hook=None):
    m = [None] * 7
    for n, p in enumerate(ORDER):
        m[p] = jnp.dot(lhs(p), rhs(p), preferred_element_type=F32)
        if hook is not None:
            hook(n)
    c12 = m[2] + m[4]
    c21 = m[1] + m[3]
    c11 = ((m[3] - m[4]) + m[6]) + m[0]
    c22 = ((m[2] - m[1]) + m[5]) + m[0]
    return c11, c12, c21, c22


def _geglu(g, u):
    c0 = np.float32(np.sqrt(2.0 / np.pi))
    c1 = np.float32(np.sqrt(2.0 / np.pi) * 0.044715)
    t = jnp.tanh(g * (c0 + c1 * (g * g)))
    return ((0.5 * g) * (1.0 + t)) * u


def _permute_columns(cols):
    lane = lax.broadcasted_iota(jnp.int32, cols[0].shape, 1)
    cols = list(cols)
    for t in range(3):
        s = 4 << t
        low = (lane & s) == 0
        for c in range(8):
            if c & (1 << t):
                continue
            a, b = cols[c], cols[c | (1 << t)]
            cols[c] = jnp.where(low, a, pltpu.roll(b, s, 1))
            cols[c | (1 << t)] = jnp.where(low, pltpu.roll(a, 128 - s, 1), b)
    return cols


def make(sub=256, att_rows=32, qslab=48, qkv_n=512, down_n=512, wo_n=512, flags=None):
    def kernel(x_hbm, wqkv_hbm, wo_hbm, wg_hbm, wu_hbm, wd_hbm, out_hbm,
               xs, xa, ha, wg_s, wu_s, wd_s, wq_s, wo_s, wdt, wqt, wot, qb, kb, vb, ob, outb,
               sem_x, sem_w, sem_a, sem_o):
        def x_copy(m):
            return pltpu.make_async_copy(x_hbm.at[pl.ds(m * BM, BM)], xs.at[pl.ds(m * BM, BM)], sem_x.at[m])

        def w_copies(j, slot):
            col = pl.ds(pl.multiple_of(j * FC, FC), FC)
            return (pltpu.make_async_copy(wg_hbm.at[:, col], wg_s.at[slot], sem_w.at[0, slot]),
                    pltpu.make_async_copy(wu_hbm.at[:, col], wu_s.at[slot], sem_w.at[1, slot]),
                    pltpu.make_async_copy(wd_hbm.at[col, :], wd_s.at[slot], sem_w.at[2, slot]))

        wq_copy = pltpu.make_async_copy(wqkv_hbm, wq_s, sem_a.at[0])

        def wo_copies():
            return [pltpu.make_async_copy(wo_hbm.at[:, pl.ds(h * HD + n * 256, 256)], wo_s.at[n, h],
                                          sem_a.at[1 + 2 * n + h])
                    for n in range(2) for h in range(2)]

        def out_copy(m, slot):
            return pltpu.make_async_copy(outb.at[slot], out_hbm.at[pl.ds(pl.multiple_of(m * BM, BM), BM)],
                                         sem_o.at[slot])

        def layernorm(m):
            def norm(r0):
                x = xs[pl.ds(r0, HM), :].astype(F32)
                xc = x - jnp.mean(x, axis=-1, keepdims=True)
                return xc * lax.rsqrt(jnp.mean(xc * xc, axis=-1, keepdims=True) + 1e-5)
            top, bot = norm(m * BM), norm(m * BM + HM)
            ops = _lhs_ops(top[:, :HD], top[:, HD:], bot[:, :HD], bot[:, HD:])
            for p in range(7):
                xa[p, pl.ds(m * HM, HM), :] = ops[p]

        def chunk_rhs(ref, slot):
            return _rhs_ops(ref[slot, :HD, :HF], ref[slot, :HD, HF:], ref[slot, HD:, :HF], ref[slot, HD:, HF:])

        def gate_up(j, r0, n, bg, bu):
            lhs = lambda p: xa[p, pl.ds(r0, n), :]
            g = _block_matmul(lhs, lambda p: bg[p])
            u = _block_matmul(lhs, lambda p: bu[p])
            ops = _lhs_ops(*[_geglu(gg, uu) for gg, uu in zip(g, u)])
            for p in range(7):
                ha[p, j, pl.ds(r0, n), :] = ops[p]

        def prep_down(j, slot):
            ops = _rhs_ops(wd_s[slot, :HF, :HD], wd_s[slot, :HF, HD:], wd_s[slot, HF:, :HD], wd_s[slot, HF:, HD:])
            for p in range(7):
                wdt[p, pl.ds(pl.multiple_of(j * HF, HF), HF), :] = ops[p]

        def prep_qkv(i, t):
            r0 = pl.multiple_of(jnp.minimum(i * qslab, HD - qslab), 16)
            quads = []
            for half in range(2):
                w = pltpu.bitcast(wq_s[pl.ds(half * HD + r0, qslab), t * D:(t + 1) * D], jnp.uint32)
                cols = _permute_columns([w[:, c * 128:(c + 1) * 128] for c in range(8)])
                quads.append(pltpu.bitcast(jnp.concatenate(cols[:4], axis=1), BF16))
                quads.append(pltpu.bitcast(jnp.concatenate(cols[4:], axis=1), BF16))
            ops = _rhs_ops(*quads)
            for p in range(7):
                wqt[t, p, pl.ds(r0, qslab), :] = ops[p]

        def prep_wo(i):
            i = jnp.minimum(i, 7)
            n, hh = i // 4, i % 4
            r0 = pl.multiple_of(hh * 32, 32)
            low = (lax.broadcasted_iota(jnp.int32, (32, 256), 0) & 4) == 0
            new = []
            for h in range(2):
                sl = [wo_s[n, h, pl.ds(c * 128 + r0, 32), :].astype(F32) for c in range(8)]
                for c in range(0, 8, 2):
                    a, b = sl[c], sl[c + 1]
                    sl[c] = jnp.where(low, a, pltpu.roll(b, 4, 0))
                    sl[c + 1] = jnp.where(low, pltpu.roll(a, 28, 0), b)
                new.append([jnp.concatenate([sl[2 * g + (e & 1)][(e >> 1) * 8:(e >> 1) * 8 + 8] for g in range(4)],
                                            axis=0) for e in range(8)])
            for e in range(4):
                ops = _rhs_ops(new[0][e], new[1][e], new[0][e + 4], new[1][e + 4])
                for p in range(7):
                    wot[p, n, pl.ds(e * 128 + r0, 32), :] = ops[p]

        first = w_copies(0, 0)
        x_copy(0).start()
        first[0].start()
        first[1].start()
        x_copy(1).start()
        x_copy(0).wait()
        layernorm(0)
        first[0].wait()
        first[1].wait()
        for m in range(2, NB):
            x_copy(m).start()
        first[2].start()
        bg, bu = chunk_rhs(wg_s, 0), chunk_rhs(wu_s, 0)
        for m in range(NB):
            if m + 1 < NB:
                x_copy(m + 1).wait()
            if m == 2:
                for c in w_copies(1, 1):
                    c.start()
            if m == 3:
                wq_copy.start()
                for c in wo_copies():
                    c.start()
            if m == NB - 1:
                first[2].wait()
                prep_down(0, 0)
            gate_up(0, m * HM, HM, bg, bu)
            if m + 1 < NB:
                layernorm(m + 1)
        wq_copy.wait()
        for c in wo_copies():
            c.wait()

        def chunk_step(j, carry):
            slot = j % 2
            for c in w_copies(j, slot):
                c.wait()

            @pl.when(j + 1 < NC)
            def _():
                for c in w_copies(j + 1, 1 - slot):
                    c.start()

            bg, bu = chunk_rhs(wg_s, slot), chunk_rhs(wu_s, slot)
            side = [lambda: prep_down(j, slot), lambda: prep_qkv(j - 1, 0), lambda: prep_qkv(j - 1, 1),
                    lambda: prep_qkv(j - 1, 2), lambda: prep_wo(j - 1)]
            nsub = S // 2 // sub
            for b in range(nsub):
                for q in range(len(side)):
                    if q * nsub // len(side) == b:
                        side[q]()
                gate_up(j, b * sub, sub, bg, bu)
            return carry

        lax.fori_loop(1, NC, chunk_step, 0)

        def attend(m, r0, n):
            lane = lax.broadcasted_iota(jnp.int32, (n, 128), 1)
            q = [qb[c, pl.ds(r0, n), :] for c in range(8)]
            logits = []
            for w in range(WIN):
                acc = None
                for c in range(8):
                    t = q[c] * kb[c, pl.ds(HALO + r0 - DIL * w, n), :]
                    acc = t if acc is None else acc + t
                for s in (1, 2):
                    acc = acc + jnp.where((lane & s) == 0, pltpu.roll(acc, 128 - s, 1), pltpu.roll(acc, s, 1))
                acc = acc * np.float32(DH ** -0.5)
                if r0 < DIL * w:
                    pos = m * BM + r0 + lax.broadcasted_iota(jnp.int32, (n, 128), 0)
                    acc = jnp.where(pos >= DIL * w, acc, np.float32(-1e9))
                logits.append(acc)
            mx = functools.reduce(jnp.maximum, logits)
            e = [jnp.exp(l - mx) for l in logits]
            inv = 1.0 / functools.reduce(lambda a, b: a + b, e)
            pr = [t * inv for t in e]
            for c in range(8):
                acc = None
                for w in range(WIN):
                    t = pr[w] * vb[c, pl.ds(HALO + r0 - DIL * w, n), :]
                    acc = t if acc is None else acc + t
                ob[c, pl.ds(r0, n), :] = acc

        def block_step(m, carry):
            slot = m % 2

            @pl.when(m >= 2)
            def _():
                out_copy(m - 2, slot).wait()

            h0 = pl.multiple_of(m * HM, HM)
            for c in range(8):
                kb[c, :HALO, :] = kb[c, BM:, :]
            tails = [vb[c, BM:, :] for c in range(8)]
            for t, (buf, off) in ((1, (kb, HALO)), (0, (qb, 0)), (2, (vb, HALO))):
                for n0 in range(0, HD, qkv_n):
                    cs = _block_matmul(lambda p: xa[p, pl.ds(h0, HM), :], lambda p: wqt[t, p, :, n0:n0 + qkv_n])
                    for qi, val in enumerate(cs):
                        for c in range(qkv_n // 128):
                            buf[(qi % 2) * 4 + n0 // 128 + c, pl.ds(off + (qi // 2) * HM, HM), :] = (
                                val[:, c * 128:(c + 1) * 128])
            for c in range(8):
                row0 = jnp.broadcast_to(vb[c, HALO:HALO + 1, :], (HALO, 128))
                vb[c, :HALO, :] = jnp.where(m == 0, row0, tails[c])

            natt = BM // att_rows
            todo = list(range(natt))
            nslots = 7 * (HD // down_n)
            gates = []
            for ni, n0 in enumerate(range(0, HD, down_n)):
                def hook(n):
                    k = ni * 7 + n
                    while todo and todo[0] * (nslots - 1) // natt <= k:
                        attend(m, todo.pop(0) * att_rows, att_rows)
                cs = _block_matmul(
                    lambda p: jnp.concatenate([ha[p, j, pl.ds(h0, HM), :] for j in range(NC)], axis=1),
                    lambda p: wdt[p, :, n0:n0 + down_n], hook)
                gates.append([d * jax.nn.sigmoid(d) for d in cs])
            gates = [jnp.concatenate([g[qi] for g in gates], axis=1) for qi in range(4)]

            quad = lambda r, h: jnp.concatenate([ob[4 * h + c, pl.ds(r * HM, HM), :] for c in range(4)], axis=1)
            oa = _lhs_ops(quad(0, 0), quad(0, 1), quad(1, 0), quad(1, 1))
            for n0 in range(0, HD, wo_n):
                def rhs(p):
                    if wo_n == 512:
                        return jnp.concatenate([wot[p, 0], wot[p, 1]], axis=1)
                    return wot[p, n0 // 256, :, n0 % 256:n0 % 256 + wo_n]
                cs = _block_matmul(lambda p: oa[p], rhs)
                for qi, val in enumerate(cs):
                    rows, cols = (qi // 2) * HM, (qi % 2) * HD + n0
                    res = xs[pl.ds(pl.multiple_of(m * BM + rows, HM), HM), cols:cols + wo_n].astype(F32)
                    outb[slot, rows:rows + HM, cols:cols + wo_n] = (
                        res + val * gates[qi][:, n0:n0 + wo_n]).astype(BF16)
            out_copy(m, slot).start()
            return carry

        for c in range(8):
            kb[c, BM:, :] = jnp.zeros((HALO, 128), F32)
            vb[c, BM:, :] = jnp.zeros((HALO, 128), F32)
        lax.fori_loop(0, NB, block_step, 0)
        out_copy(NB - 2, 0).wait()
        out_copy(NB - 1, 1).wait()

    def fn(A_x, A_wqkv, A_wo, B_x, B_w_gate, B_w_up, B_w_down):
        any_spec = pl.BlockSpec(memory_space=pl.ANY)
        out = pl.pallas_call(
            kernel,
            in_specs=[any_spec] * 6,
            out_specs=any_spec,
            out_shape=jax.ShapeDtypeStruct((S, D), BF16),
            scratch_shapes=[
                pltpu.VMEM((S, D), BF16),
                pltpu.VMEM((7, S // 2, HD), BF16),
                pltpu.VMEM((7, NC, S // 2, HF), BF16),
                pltpu.VMEM((2, D, FC), BF16),
                pltpu.VMEM((2, D, FC), BF16),
                pltpu.VMEM((2, FC, D), BF16),
                pltpu.VMEM((D, 3 * D), BF16),
                pltpu.VMEM((2, 2, D, 256), BF16),
                pltpu.VMEM((7, F // 2, HD), BF16),
                pltpu.VMEM((3, 7, HD, HD), BF16),
                pltpu.VMEM((7, 2, HD, 256), BF16),
                pltpu.VMEM((8, BM, 128), F32),
                pltpu.VMEM((8, HALO + BM, 128), F32),
                pltpu.VMEM((8, HALO + BM, 128), F32),
                pltpu.VMEM((8, BM, 128), F32),
                pltpu.VMEM((2, BM, D), BF16),
                pltpu.SemaphoreType.DMA((NB,)),
                pltpu.SemaphoreType.DMA((3, 2)),
                pltpu.SemaphoreType.DMA((5,)),
                pltpu.SemaphoreType.DMA((2,)),
            ],
            compiler_params=pltpu.CompilerParams(vmem_limit_bytes=120 * 2**20, flags=flags),
        )(A_x.reshape(S, D), A_wqkv, A_wo, B_w_gate, B_w_up, B_w_down)
        return out.reshape(1, S, D)

    return fn


@jax.jit
def pallas_recurrent_scan__sliding_local_dilated__geglu_ffn__prompt_kernel(
        A_x, A_wqkv, A_wo, B_x, B_w_gate, B_w_up, B_w_down):
    return make()(A_x, A_wqkv, A_wo, B_x, B_w_gate, B_w_up, B_w_down)
```

```python
import contextlib
import functools
import numpy as np
import jax
import jax.numpy as jnp
from jax import lax
from jax.experimental import pallas as pl
from jax.experimental.pallas import tpu as pltpu

S, D, F = 2048, 1024, 3584
DH, WIN, DIL = 32, 8, 2
BM = 256
HM = BM // 2
NB = S // BM
FC = 256
HF = FC // 2
NC = F // FC
HD = D // 2
NQ = 12
EV = {"XLA_TPU_EVENLY_DISTRIBUTE_CRITICAL_NODES": True}
HALO = 16
HS = S // 2
F32, BF16, U32 = jnp.float32, jnp.bfloat16, jnp.uint32


def _pack(v):
    return pltpu.bitcast(v.astype(BF16), U32)


def _unpack(v):
    return pltpu.bitcast(v, BF16)


def _rows(start, n):
    return pl.ds(start // 2, n // 2)


def _shifted(ref, rows, limit):
    return ref.at[pl.ds(pl.multiple_of(rows // 2 if isinstance(rows, int) else rows >> 1, 8), ref.shape[0] - limit // 2)]


def _lhs_ops(a11, a12, a21, a22):
    return [_pack(o) for o in (a11 + a22, a21 + a22, a11, a22, a11 + a12, a21 - a11, a12 - a22)]


def _rhs_ops(b11, b12, b21, b22):
    f11, f12, f21, f22 = (b.astype(F32) for b in (b11, b12, b21, b22))
    return [_pack(o) for o in (f11 + f22, b11, f12 - f22, f21 - f11, b22, f11 + f12, f21 + f22)]


def _rhs_op(p, quad):
    first, sign, second = ((0, 1, 3), (0, 0, 0), (1, -1, 3), (2, -1, 0), (3, 0, 0), (0, 1, 1), (2, 1, 3))[p]
    if sign == 0:
        return _pack(quad(first))
    a, b = quad(first).astype(F32), quad(second).astype(F32)
    return _pack(a + b if sign > 0 else a - b)


def _geglu(g, u):
    c0 = np.float32(np.sqrt(2.0 / np.pi))
    c1 = np.float32(np.sqrt(2.0 / np.pi) * 0.044715)
    t = jnp.tanh(g * (c0 + c1 * (g * g)))
    return ((0.5 * g) * (1.0 + t)) * u


def _silu(d):
    h = 0.5 * d
    return h * (1.0 + jnp.tanh(h))


def _permute_columns(cols):
    lane = lax.broadcasted_iota(jnp.int32, cols[0].shape, 1)
    cols = list(cols)
    for t in range(3):
        s = 4 << t
        low = (lane & s) == 0
        for c in range(8):
            if c & (1 << t):
                continue
            a, b = cols[c], cols[c | (1 << t)]
            cols[c] = jnp.where(low, a, pltpu.roll(b, s, 1))
            cols[c | (1 << t)] = jnp.where(low, pltpu.roll(a, 128 - s, 1), b)
    return cols


class _Jobs:
    def __init__(self, jobs, slots, first=0):
        self.jobs, self.slots, self.first, self.done, self.tick = list(jobs), slots, first, 0, 0

    def __call__(self):
        self.tick += 1
        while self.done < len(self.jobs) and self.done * self.slots < (self.tick - self.first) * len(self.jobs):
            self.jobs[self.done]()
            self.done += 1

    def finish(self):
        for job in self.jobs[self.done:]:
            job()
        self.done = len(self.jobs)


def make(scopes=False, sub=256, att_rows=16, qkv_n=512, down_n=512, wo_n=512, flags=EV, gather=True,
         order=(1, 4, 2, 3, 5, 6, 0), ln_rows=16, att_first=7, att_slots=13, side_frac=0.8, nobc=False, qkv_order=(2, 1, 0)):
    scope = jax.named_scope if scopes else (lambda n: contextlib.nullcontext())

    def scoped(name, f):
        def g(*a):
            with scope(name):
                return f(*a)
        return g

    def _block_matmul(lhs, rhs, hook=None):
        m = [None] * 7
        for p in order:
            m[p] = jnp.dot(_unpack(lhs(p)), _unpack(rhs(p)), preferred_element_type=F32)
            if hook is not None:
                hook()
        c12 = m[2] + m[4]
        c21 = m[1] + m[3]
        c11 = ((m[3] - m[4]) + m[6]) + m[0]
        c22 = ((m[2] - m[1]) + m[5]) + m[0]
        return c11, c12, c21, c22

    def kernel(x_hbm, wqkv_hbm, wo_hbm, wg_hbm, wu_hbm, wd_hbm, out_hbm,
               xs, xa, ha, wg_s, wu_s, wd_s, wq_s, wo_s, wgt, wut, wdt, wqt, wot, qb, kb, vb, ob, oa, outb,
               sem_x, sem_w, sem_a, sem_o):
        def x_copy(m):
            return pltpu.make_async_copy(x_hbm.at[pl.ds(m * BM, BM)], xs.at[pl.ds(m * BM, BM)], sem_x.at[m])

        def w_copies(j, slot):
            col = pl.ds(pl.multiple_of(j * FC, FC), FC)
            return (pltpu.make_async_copy(wg_hbm.at[:, col], wg_s.at[slot], sem_w.at[0, slot]),
                    pltpu.make_async_copy(wu_hbm.at[:, col], wu_s.at[slot], sem_w.at[1, slot]),
                    pltpu.make_async_copy(wd_hbm.at[col, :], wd_s.at[slot], sem_w.at[2, slot]))

        def wq_copies(i):
            cols = pl.ds(pl.multiple_of((i >> 2) * D, D), D)
            return [pltpu.make_async_copy(wqkv_hbm.at[pl.ds(pl.multiple_of(h * HD + (i & 3) * 128, 128), 128), cols],
                                          wq_s.at[i, h], sem_w.at[3 + h, i & 1]) for h in range(2)]

        def wo_copies(n):
            return [pltpu.make_async_copy(wo_hbm.at[:, pl.ds(h * HD + n * 256, 256)], wo_s.at[n, h],
                                          sem_a.at[n, h]) for h in range(2)]

        def out_copy(m, slot):
            return pltpu.make_async_copy(outb.at[slot], out_hbm.at[pl.ds(pl.multiple_of(m * BM, BM), BM)],
                                         sem_o.at[slot])

        def layernorm(m, r):
            def norm(r0):
                x = xs[pl.ds(r0, ln_rows), :].astype(F32)
                xc = x - jnp.mean(x, axis=-1, keepdims=True)
                return xc * lax.rsqrt(jnp.mean(xc * xc, axis=-1, keepdims=True) + 1e-5)
            top, bot = norm(m * BM + r), norm(m * BM + HM + r)
            ops = _lhs_ops(top[:, :HD], top[:, HD:], bot[:, :HD], bot[:, HD:])
            for p in range(7):
                xa[_rows(p * HS + m * HM + r, ln_rows), :] = ops[p]

        def ln_jobs(m):
            return [functools.partial(layernorm, m, r) for r in range(0, HM, ln_rows)]

        def chunk_rhs(src, dst, slot, fresh, p):
            if not fresh:
                return dst[:, p * HF:(p + 1) * HF]
            quad = lambda q: src.at[slot][(q // 2) * HD:(q // 2 + 1) * HD, (q % 2) * HF:(q % 2 + 1) * HF]
            val = _rhs_op(p, quad)
            dst[:, p * HF:(p + 1) * HF] = val
            return val

        def gate_up(j, slot, r0, n, hook, mid=None):
            lhs = lambda p: xa[_rows(p * HS + r0, n), :]
            g = _block_matmul(lhs, functools.partial(chunk_rhs, wg_s, wgt, slot, r0 == 0), hook)
            if mid is not None:
                mid()
            u = _block_matmul(lhs, functools.partial(chunk_rhs, wu_s, wut, slot, r0 == 0), hook)
            ops = _lhs_ops(*[_geglu(gg, uu) for gg, uu in zip(g, u)])
            for p in range(7):
                _shifted(ha, j * HS, (NC - 1) * HS)[_rows(r0, n), p * HF:(p + 1) * HF] = ops[p]

        def prep_down(j, slot, r):
            top, bot = wd_s.at[slot][r:r + 16, :], wd_s.at[slot][HF + r:HF + r + 16, :]
            ops = _rhs_ops(top[:, :HD], top[:, HD:], bot[:, :HD], bot[:, HD:])
            for p in range(7):
                _shifted(wdt, j * HF, (NC - 1) * HF)[_rows(p * (F // 2) + r, 16), :] = ops[p]

        def prep_qkv(i, r):
            quads = []
            for h in range(2):
                w = pltpu.bitcast(wq_s[i, h, r:r + 16, :], U32)
                cols = _permute_columns([w[:, c * 128:(c + 1) * 128] for c in range(8)])
                quads.append(_unpack(jnp.concatenate(cols[:4], axis=1)))
                quads.append(_unpack(jnp.concatenate(cols[4:], axis=1)))
            ops = _rhs_ops(*quads)
            for p in range(7):
                _shifted(wqt, i * 128, (NQ - 1) * 128)[_rows(p * 3 * HD + r, 16), :] = ops[p]

        def prep_wo(i, c0, g2):
            n, r0 = i >> 2, pl.multiple_of((i & 3) * 32, 32)
            low = (lax.broadcasted_iota(jnp.int32, (32, 128), 0) & 4) == 0
            new = []
            for h in range(2):
                sl = [wo_s.at[n, :, pl.ds(r0, D - 96)][h, pl.ds((4 * g2 + c) * 128, 32), c0:c0 + 128].astype(F32) for c in range(4)]
                for c in (0, 2):
                    a, b = sl[c], sl[c + 1]
                    sl[c] = jnp.where(low, a, pltpu.roll(b, 4, 0))
                    sl[c + 1] = jnp.where(low, pltpu.roll(a, 28, 0), b)
                new.append([jnp.concatenate([sl[2 * g + (e & 1)][(e >> 1) * 8:(e >> 1) * 8 + 8] for g in range(2)],
                                            axis=0) for e in range(8)])
            for e in range(4):
                ops = _rhs_ops(new[0][e], new[1][e], new[0][e + 4], new[1][e + 4])
                for p in range(7):
                    _shifted(wot, n * HD + r0, HD + 96)[_rows(p * D + e * 128 + 16 * g2, 16), c0:c0 + 128] = ops[p]

        first, second, wo0 = w_copies(0, 0), w_copies(1, 1), wo_copies(0)
        x_copy(0).start()
        first[0].start()
        first[1].start()
        x_copy(1).start()
        with scope('w_x0'):
            x_copy(0).wait()
        x_copy(2).start()
        with scope('ln0'):
            for job in ln_jobs(0):
                job()
        with scope('w_wg'):
            first[0].wait()
            first[1].wait()
            x_copy(1).wait()
        later = {0: [x_copy(3), x_copy(4)], 1: [x_copy(5), x_copy(6), x_copy(7), first[2]],
                 2: [*second], 4: [*wq_copies(0), *wo0]}
        waits = {1: [x_copy(2)], 2: [x_copy(3), x_copy(4)], 4: [x_copy(5), x_copy(6), x_copy(7), first[2]]}
        for m in range(NB):
            with scope('p0_w'):
                for c in waits.get(m, []):
                    c.wait()
            for c in later.get(m, []):
                c.start()
            jobs = _Jobs(ln_jobs(m + 1) if m + 1 < NB else
                         [functools.partial(prep_down, 0, 0, r) for r in range(0, HF, 16)], 11)
            gate_up(0, 0, m * HM, HM, jobs)
            jobs.finish()
        with scope('w_end'):
            for c in wo0:
                c.wait()

        def chunk_step(j, carry):
            slot = j & 1
            for c in w_copies(j, slot):
                c.wait()

            @pl.when(j - 1 < NQ)
            def _():
                for c in wq_copies(j - 1):
                    c.wait()

            @pl.when(j == 5)
            def _():
                for c in wo_copies(1):
                    c.wait()

            @pl.when(j + 1 < NC)
            def _():
                for c in w_copies(j + 1, 1 - slot):
                    c.start()

            @pl.when(j < NQ)
            def _():
                for c in wq_copies(j):
                    c.start()

            @pl.when(j == 4)
            def _():
                for c in wo_copies(1):
                    c.start()

            iq, io = jnp.minimum(j - 1, NQ - 1), jnp.minimum(j - 1, 7)
            side = []
            for r in range(8):
                side.append(functools.partial(prep_qkv, iq, r * 16))
                side.append(functools.partial(prep_down, j, slot, r * 16))
                if r % 2:
                    side.append(functools.partial(prep_wo, io, (r // 4) * 128, (r // 2) % 2))
            nsub = S // 2 // sub
            jobs = _Jobs(side, int(nsub * 14 * side_frac), 7)
            for b in range(nsub):
                gate_up(j, slot, b * sub, sub, jobs)
            jobs.finish()
            return carry

        with scope('p1'):
            lax.fori_loop(1, NC, scoped('p1_it', chunk_step), 0)

        def attend(m, r0, n):
            lane = lax.broadcasted_iota(jnp.int32, (n, 128), 1)
            logits = []
            for w in range(WIN):
                acc = None
                for c in range(8):
                    t = qb[c, pl.ds(r0, n), :] * kb[c, pl.ds(HALO + r0 - DIL * w, n), :]
                    acc = t if acc is None else acc + t
                for s in (1, 2):
                    if gather:
                        acc = acc + jnp.take_along_axis(acc, lane ^ s, axis=1)
                    else:
                        acc = acc + jnp.where((lane & s) == 0, pltpu.roll(acc, 128 - s, 1), pltpu.roll(acc, s, 1))
                acc = acc * np.float32(DH ** -0.5)
                if r0 < DIL * w:
                    pos = m * BM + r0 + lax.broadcasted_iota(jnp.int32, (n, 128), 0)
                    acc = jnp.where(pos >= DIL * w, acc, np.float32(-1e9))
                logits.append(acc)
            mx = functools.reduce(jnp.maximum, logits)
            e = [jnp.exp(l - mx) for l in logits]
            inv = 1.0 / functools.reduce(lambda a, b: a + b, e)
            pr = [t * inv for t in e]
            for c in range(8):
                acc = None
                for w in range(WIN):
                    t = pr[w] * vb[c, pl.ds(HALO + r0 - DIL * w, n), :]
                    acc = t if acc is None else acc + t
                ob[c, pl.ds(r0, n), :] = acc

        def pack_o(r0, n):
            for c in range(4):
                ops = _lhs_ops(ob[c, pl.ds(r0, n), :], ob[4 + c, pl.ds(r0, n), :],
                               ob[c, pl.ds(HM + r0, n), :], ob[4 + c, pl.ds(HM + r0, n), :])
                for p in range(7):
                    oa[_rows(p * HM + r0, n), c * 128:(c + 1) * 128] = ops[p]

        def block_step(m, carry):
            slot = m & 1

            @pl.when(m >= 2)
            def _():
                out_copy(m - 2, slot).wait()

            h0 = m * HM
            for c in range(8):
                kb[c, :HALO, :] = kb[c, BM:, :]
                vb[c, :HALO, :] = vb[c, BM:, :]
            for t in qkv_order:
                buf, off = ((qb, 0), (kb, HALO), (vb, HALO))[t]
                for n0 in range(0, HD, qkv_n):
                    cs = _block_matmul(lambda p: _shifted(xa, h0, HS - HM)[_rows(p * HS, HM), :],
                                       lambda p: wqt[_rows((p * 3 + t) * HD, HD), n0:n0 + qkv_n])
                    for qi, val in enumerate(cs):
                        for c in range(qkv_n // 128):
                            buf[(qi % 2) * 4 + n0 // 128 + c, pl.ds(off + (qi // 2) * HM, HM), :] = (
                                val[:, c * 128:(c + 1) * 128])
                if t == 2:
                    for c in range(8):
                        row0 = jnp.broadcast_to(vb[c, HALO:HALO + 1, :], (HALO, 128))
                        vb[c, :HALO, :] = jnp.where(m == 0, row0, vb[c, :HALO, :])

            todo = []
            for r in range(0, HM, att_rows):
                todo.append(functools.partial(attend, m, r, att_rows))
                todo.append(functools.partial(attend, m, HM + r, att_rows))
                if (r + att_rows) % 16 == 0:
                    n = max(16, att_rows)
                    todo.append(functools.partial(pack_o, r + att_rows - n, n))
            nslots = 7 * (HD // down_n)
            jobs = _Jobs(todo, max(nslots - 1 - nslots // 7, 1))
            gates = []
            for n0 in range(0, HD, down_n):
                cs = _block_matmul(
                    lambda p: jnp.concatenate([_shifted(ha, h0, HS - HM)[_rows(j * HS, HM), p * HF:(p + 1) * HF] for j in range(NC)], axis=1),
                    lambda p: wdt[_rows(p * (F // 2), F // 2), n0:n0 + down_n], jobs)
                gates.append([_silu(d) for d in cs])
            jobs.finish()
            gates = [jnp.concatenate([g[qi] for g in gates], axis=1) for qi in range(4)]

            for n0 in range(0, HD, wo_n):
                def rhs(p):
                    if wo_n == 512:
                        return jnp.concatenate([wot[_rows(p * D + n * HD, HD), :] for n in range(2)], axis=1)
                    return wot[_rows(p * D + (n0 // 256) * HD, HD), n0 % 256:n0 % 256 + wo_n]
                cs = _block_matmul(lambda p: oa[_rows(p * HM, HM), :], rhs)
                for qi, val in enumerate(cs):
                    rows, cols = (qi // 2) * HM, (qi % 2) * HD + n0
                    res = xs[pl.ds(pl.multiple_of(m * BM + rows, HM), HM), cols:cols + wo_n].astype(F32)
                    outb[slot, rows:rows + HM, cols:cols + wo_n] = (
                        res + val * gates[qi][:, n0:n0 + wo_n]).astype(BF16)
            out_copy(m, slot).start()
            return carry

        for c in range(8):
            kb[c, BM:, :] = jnp.zeros((HALO, 128), F32)
            vb[c, BM:, :] = jnp.zeros((HALO, 128), F32)
        with scope('p2'):
            lax.fori_loop(0, NB, scoped('p2_it', block_step), 0)
        with scope('tail'):
            out_copy(NB - 2, 0).wait()
            out_copy(NB - 1, 1).wait()

    def fn(A_x, A_wqkv, A_wo, B_x, B_w_gate, B_w_up, B_w_down):
        any_spec = pl.BlockSpec(memory_space=pl.ANY)
        out = pl.pallas_call(
            kernel,
            in_specs=[any_spec] * 6,
            out_specs=any_spec,
            out_shape=jax.ShapeDtypeStruct((S, D), BF16),
            scratch_shapes=[
                pltpu.VMEM((S, D), BF16),
                pltpu.VMEM((7 * HS // 2, HD), U32),
                pltpu.VMEM((NC * HS // 2, 7 * HF), U32),
                pltpu.VMEM((2, D, FC), BF16),
                pltpu.VMEM((2, D, FC), BF16),
                pltpu.VMEM((2, FC, D), BF16),
                pltpu.VMEM((NQ, 2, 128, D), BF16),
                pltpu.VMEM((2, 2, D, 256), BF16),
                pltpu.VMEM((HD // 2, 7 * HF), U32),
                pltpu.VMEM((HD // 2, 7 * HF), U32),
                pltpu.VMEM((7 * F // 4, HD), U32),
                pltpu.VMEM((21 * HD // 2, HD), U32),
                pltpu.VMEM((7 * HD, 256), U32),
                pltpu.VMEM((8, BM, 128), F32),
                pltpu.VMEM((8, HALO + BM, 128), F32),
                pltpu.VMEM((8, HALO + BM, 128), F32),
                pltpu.VMEM((8, BM, 128), F32),
                pltpu.VMEM((7 * HM // 2, HD), U32),
                pltpu.VMEM((2, BM, D), BF16),
                pltpu.SemaphoreType.DMA((NB,)),
                pltpu.SemaphoreType.DMA((5, 2)),
                pltpu.SemaphoreType.DMA((2, 2)),
                pltpu.SemaphoreType.DMA((2,)),
            ],
            compiler_params=pltpu.CompilerParams(vmem_limit_bytes=120 * 2**20, flags=flags,
                                                 disable_bounds_checks=nobc),
        )(A_x.reshape(S, D), A_wqkv, A_wo, B_w_gate, B_w_up, B_w_down)
        return out.reshape(1, S, D)

    return fn


@jax.jit
def pallas_recurrent_scan__sliding_local_dilated__geglu_ffn__prompt_kernel(
        A_x, A_wqkv, A_wo, B_x, B_w_gate, B_w_up, B_w_down):
    return make(sub=512)(A_x, A_wqkv, A_wo, B_x, B_w_gate, B_w_up, B_w_down)
```

```python
import contextlib
import functools
import numpy as np
import jax
import jax.numpy as jnp
from jax import lax
from jax.experimental import pallas as pl
from jax.experimental.pallas import tpu as pltpu

S, D, F = 2048, 1024, 3584
DH, WIN, DIL = 32, 8, 2
BM = 256
HM = BM // 2
NB = S // BM
FC = 256
HF = FC // 2
NC = F // FC
HD = D // 2
HS = S // 2
NQ = 12
HALO = 16
EV = {"XLA_TPU_EVENLY_DISTRIBUTE_CRITICAL_NODES": True}
F32, BF16, U32 = jnp.float32, jnp.bfloat16, jnp.uint32


def _pack(v):
    return pltpu.bitcast(v.astype(BF16), U32)


def _unpack(v):
    return pltpu.bitcast(v, BF16)


def _rows(start, n):
    return pl.ds(start // 2, n // 2)


def _shifted(ref, rows, limit):
    start = rows // 2 if isinstance(rows, int) else pl.multiple_of(rows >> 1, 8)
    return ref.at[pl.ds(start, ref.shape[0] - limit // 2)]


def _lhs_ops(a11, a12, a21, a22):
    return [_pack(o) for o in (a11 + a22, a21 + a22, a11, a22, a11 + a12, a21 - a11, a12 - a22)]


def _rhs_ops(b11, b12, b21, b22):
    return [_pack(o) for o in (b11 + b22, b11, b12 - b22, b21 - b11, b22, b11 + b12, b21 + b22)]


def _rhs_op(p, quad):
    first, sign, second = ((0, 1, 3), (0, 0, 0), (1, -1, 3), (2, -1, 0), (3, 0, 0), (0, 1, 1), (2, 1, 3))[p]
    if sign == 0:
        return _pack(quad(first))
    a, b = quad(first).astype(F32), quad(second).astype(F32)
    return _pack(a + b if sign > 0 else a - b)


def _geglu(g, u):
    c0 = np.float32(np.sqrt(2.0 / np.pi))
    c1 = np.float32(np.sqrt(2.0 / np.pi) * 0.044715)
    t = jnp.tanh(g * (c0 + c1 * (g * g)))
    return ((0.5 * g) * (1.0 + t)) * u


def _silu(d):
    h = 0.5 * d
    return h * (1.0 + jnp.tanh(h))


def _permute_columns(cols):
    lane = lax.broadcasted_iota(jnp.int32, cols[0].shape, 1)
    cols = list(cols)
    for t in range(3):
        s = 4 << t
        low = (lane & s) == 0
        for c in range(8):
            if c & (1 << t):
                continue
            a, b = cols[c], cols[c | (1 << t)]
            cols[c] = jnp.where(low, a, pltpu.roll(b, s, 1))
            cols[c | (1 << t)] = jnp.where(low, pltpu.roll(a, 128 - s, 1), b)
    return cols


def _after(anchor, v):
    if anchor is None:
        return v
    a = jnp.tile(anchor, (v.shape[0] // 8, v.shape[1] // 128))
    return jnp.where(jnp.abs(a) < 0, jnp.zeros_like(v), v)


def _tiles(products):
    return [(m, r, c) for m in products for c in range(0, m.shape[1], 128) for r in range(0, m.shape[0], 8)]


def _spread(jobs, products, lo, hi):
    tiles = _tiles(products)
    for n, job in enumerate(jobs):
        k = int(np.floor((lo + (hi - lo) * n / len(jobs)) * len(tiles)))
        if k < 0:
            job(None)
        else:
            m, r, c = tiles[k]
            job(m[r:r + 8, c:c + 128])


def make(scopes=False, sub=512, att_rows=8, qkv_n=512, down_n=512, flags=EV,
         order=(1, 4, 2, 3, 5, 6, 0), ln_rows=16, nobc=False, nosc=False, att=(-0.03, 0.7), side=(0.3, 0.9),
         ln=(-0.1, 0.65), gate_q=False, p0=0, corder=((4, 5, 6, 7, 0, 1, 2, 3), range(8))):
    scope = jax.named_scope if scopes else (lambda n: contextlib.nullcontext())

    def scoped(name, f):
        def g(*a):
            with scope(name):
                return f(*a)
        return g

    def _block_matmul(lhs, rhs, seen=None):
        m = [None] * 7
        for p in order:
            m[p] = jnp.dot(_unpack(lhs(p)), _unpack(rhs(p)), preferred_element_type=F32)
            if seen is not None:
                seen.append(m[p])
        c12 = m[2] + m[4]
        c21 = m[1] + m[3]
        c11 = ((m[3] - m[4]) + m[6]) + m[0]
        c22 = ((m[2] - m[1]) + m[5]) + m[0]
        return c11, c12, c21, c22

    def kernel(x_hbm, wqkv_hbm, wo_hbm, wg_hbm, wu_hbm, wd_hbm, out_hbm,
               xs, xa, ha, wg_s, wu_s, wd_s, wq_s, wo_s, wgt, wut, wdt, wqt, wot, qb, kb, vb, ob, oa, outb,
               sem_x, sem_w, sem_a, sem_o):
        def x_copy(m):
            return pltpu.make_async_copy(x_hbm.at[pl.ds(m * BM, BM)], xs.at[pl.ds(m * BM, BM)], sem_x.at[m])

        def w_copies(j, slot):
            col = pl.ds(pl.multiple_of(j * FC, FC), FC)
            return (pltpu.make_async_copy(wg_hbm.at[:, col], wg_s.at[slot], sem_w.at[0, slot]),
                    pltpu.make_async_copy(wu_hbm.at[:, col], wu_s.at[slot], sem_w.at[1, slot]),
                    pltpu.make_async_copy(wd_hbm.at[col, :], wd_s.at[slot], sem_w.at[2, slot]))

        def wq_copies(i):
            cols = pl.ds(pl.multiple_of((i >> 2) * D, D), D)
            return [pltpu.make_async_copy(wqkv_hbm.at[pl.ds(pl.multiple_of(h * HD + (i & 3) * 128, 128), 128), cols],
                                          wq_s.at[i, h], sem_w.at[3 + h, i & 1]) for h in range(2)]

        def wo_copies(n):
            return [pltpu.make_async_copy(wo_hbm.at[:, pl.ds(h * HD + n * 256, 256)], wo_s.at[n, h],
                                          sem_a.at[n, h]) for h in range(2)]

        def out_copy(m, slot):
            return pltpu.make_async_copy(outb.at[slot], out_hbm.at[pl.ds(pl.multiple_of(m * BM, BM), BM)],
                                         sem_o.at[slot])

        def layernorm(m, r, anchor):
            def norm(r0):
                x = xs[pl.ds(r0, ln_rows), :].astype(F32)
                x = jnp.concatenate([_after(anchor, x[:, :128]), x[:, 128:]], axis=1)
                xc = x - jnp.mean(x, axis=-1, keepdims=True)
                return xc * lax.rsqrt(jnp.mean(xc * xc, axis=-1, keepdims=True) + 1e-5)
            top, bot = norm(m * BM + r), norm(m * BM + HM + r)
            ops = _lhs_ops(top[:, :HD], top[:, HD:], bot[:, :HD], bot[:, HD:])
            for p in range(7):
                xa[_rows(p * HS + m * HM + r, ln_rows), :] = ops[p]

        def ln_jobs(m):
            return [functools.partial(layernorm, m, r) for r in range(0, HM, ln_rows)]

        def chunk_rhs(src, dst, slot, fresh, p):
            if fresh:
                dst[:, p * HF:(p + 1) * HF] = _rhs_op(
                    p, lambda q: src.at[slot][(q // 2) * HD:(q // 2 + 1) * HD, (q % 2) * HF:(q % 2 + 1) * HF])
            return dst[:, p * HF:(p + 1) * HF]

        def gate_up(j, slot, r0, n, mid=None):
            seen = []
            lhs = lambda p: xa[_rows(p * HS + r0, n), :]
            g = _block_matmul(lhs, functools.partial(chunk_rhs, wg_s, wgt, slot, r0 == 0), seen)
            if mid is not None:
                mid()
            u = _block_matmul(lhs, functools.partial(chunk_rhs, wu_s, wut, slot, r0 == 0), seen)
            ops = _lhs_ops(*[_geglu(gg, uu) for gg, uu in zip(g, u)])
            for p in range(7):
                _shifted(ha, j * HS, (NC - 1) * HS)[_rows(r0, n), p * HF:(p + 1) * HF] = ops[p]
            return seen

        def prep_down(j, slot, r, anchor):
            top = wd_s.at[slot][r:r + 16, :].astype(F32)
            bot = wd_s.at[slot][HF + r:HF + r + 16, :].astype(F32)
            ops = _rhs_ops(_after(anchor, top[:, :HD]), top[:, HD:], bot[:, :HD], _after(anchor, bot[:, HD:]))
            for p in range(7):
                _shifted(wdt, j * HF, (NC - 1) * HF)[_rows(p * (F // 2) + r, 16), :] = ops[p]

        def prep_qkv(i, r, anchor):
            quads = []
            for h in range(2):
                w = pltpu.bitcast(wq_s.at[i][h, r:r + 16, :], U32)
                if gate_q:
                    w = _after(anchor, w)
                cols = _permute_columns([w[:, c * 128:(c + 1) * 128] for c in range(8)])
                quads.append(_unpack(jnp.concatenate(cols[:4], axis=1)).astype(F32))
                quads.append(_unpack(jnp.concatenate(cols[4:], axis=1)).astype(F32))
            ops = _rhs_ops(*quads)
            for p in range(7):
                _shifted(wqt, i * 128, (NQ - 1) * 128)[_rows(p * 3 * HD + r, 16), :] = ops[p]

        def prep_wo(i, c0, g2, e2, anchor):
            n, r0 = i >> 2, pl.multiple_of((i & 3) * 32, 32)
            low = lax.broadcasted_iota(jnp.int32, (8, 128), 0) < 4
            src = wo_s.at[n, :, pl.ds(r0, D - 96)]
            new = {}
            for h in range(2):
                for e in (e2, e2 + 2):
                    t = [_after(anchor, src[h, pl.ds((4 * g2 + c) * 128 + e * 8, 8), c0:c0 + 128].astype(F32))
                         for c in range(4)]
                    new[h, 2 * e] = jnp.concatenate(
                        [jnp.where(low, t[c], pltpu.roll(t[c + 1], 4, 0)) for c in (0, 2)], axis=0)
                    new[h, 2 * e + 1] = jnp.concatenate(
                        [jnp.where(low, pltpu.roll(t[c], 4, 0), t[c + 1]) for c in (0, 2)], axis=0)
            for e in (2 * e2, 2 * e2 + 1):
                ops = _rhs_ops(new[0, e], new[1, e], new[0, e + 4], new[1, e + 4])
                for p in range(7):
                    _shifted(wot, n * HD + r0, HD + 96)[_rows(p * D + e * 128 + 16 * g2, 16), c0:c0 + 128] = ops[p]

        first, second, wo0 = w_copies(0, 0), w_copies(1, 1), wo_copies(0)
        for c in (x_copy(0), x_copy(1), first[0], first[1], x_copy(2)):
            c.start()
        for m in range(2):
            with scope('w_x'):
                x_copy(m).wait()
            x_copy(3 + m).start()
            for job in ln_jobs(m):
                job(None)
        with scope('w_wg'):
            first[0].wait()
        x_copy(5).start()

        def arrive():
            with scope('w_wu'):
                first[1].wait()
                x_copy(2).wait()
            for c in (x_copy(6), x_copy(7), first[2]):
                c.start()

        seen = gate_up(0, 0, 0, 2 * HM, arrive)
        _spread(ln_jobs(2), seen[7:], *ln)
        for m in range(2, NB):
            if m in (2, 4):
                with scope('p0_w'):
                    for c in ((x_copy(3), x_copy(4)) if m == 2 else (x_copy(5), x_copy(6), x_copy(7), first[2])):
                        c.wait()
                for c in (second if m == 2 else (*wq_copies(0), *wo0)):
                    c.start()
            seen = gate_up(0, 0, m * HM, HM)
            _spread(ln_jobs(m + 1) if m + 1 < NB else
                    [functools.partial(prep_down, 0, 0, r) for r in range(0, HF, 16)], seen,
                    *(ln if m in (2, 4) else (max(ln[0], 0), ln[1])))
        with scope('w_end'):
            for c in wo0:
                c.wait()

        def chunk_step(j, carry):
            slot = j & 1
            for c in w_copies(j, slot):
                c.wait()

            @pl.when(j - 1 < NQ)
            def _():
                for c in wq_copies(j - 1):
                    c.wait()

            @pl.when(j == 5)
            def _():
                for c in wo_copies(1):
                    c.wait()

            @pl.when(j + 1 < NC)
            def _():
                for c in w_copies(j + 1, 1 - slot):
                    c.start()

            @pl.when(j < NQ)
            def _():
                for c in wq_copies(j):
                    c.start()

            @pl.when(j == 4)
            def _():
                for c in wo_copies(1):
                    c.start()

            iq, io = jnp.minimum(j - 1, NQ - 1), jnp.minimum(j - 1, 7)
            jobs = []
            for r in range(8):
                jobs.append(functools.partial(prep_qkv, iq, r * 16))
                jobs.append(functools.partial(prep_down, j, slot, r * 16))
                jobs.append(functools.partial(prep_wo, io, (r // 4) * 128, (r // 2) % 2, r % 2))
            seen = []
            for r0 in range(0, HS, sub):
                seen += gate_up(j, slot, r0, sub)
            _spread(jobs, seen, *side)
            return carry

        with scope('p1'):
            lax.fori_loop(1, NC, scoped('p1_it', chunk_step), 0)

        def attend(m, r0, n, anchor):
            lane = lax.broadcasted_iota(jnp.int32, (n, 128), 1)
            logits = []
            q = [_after(anchor, qb[c, pl.ds(r0, n), :]) for c in range(8)]
            for w in range(WIN):
                acc = None
                for c in (corder[0] if r0 < HM else corder[1]):
                    t = q[c] * kb[c, pl.ds(HALO + r0 - DIL * w, n), :]
                    acc = t if acc is None else acc + t
                for s in (1, 2):
                    acc = acc + jnp.take_along_axis(acc, lane ^ s, axis=1)
                acc = acc * np.float32(DH ** -0.5)
                if r0 < DIL * w:
                    pos = m * BM + r0 + lax.broadcasted_iota(jnp.int32, (n, 128), 0)
                    acc = jnp.where(pos >= DIL * w, acc, np.float32(-1e9))
                logits.append(acc)
            mx = functools.reduce(jnp.maximum, logits)
            e = [jnp.exp(l - mx) for l in logits]
            inv = 1.0 / functools.reduce(lambda a, b: a + b, e)
            pr = [t * inv for t in e]
            for c in range(8):
                acc = None
                for w in range(WIN):
                    t = pr[w] * vb[c, pl.ds(HALO + r0 - DIL * w, n), :]
                    acc = t if acc is None else acc + t
                ob[c, pl.ds(r0, n), :] = acc

        def block_step(m, carry):
            slot = m & 1

            @pl.when(m >= 2)
            def _():
                out_copy(m - 2, slot).wait()

            h0 = m * HM
            for c in range(8):
                kb[c, :HALO, :] = kb[c, BM:, :]
                vb[c, :HALO, :] = vb[c, BM:, :]
            for t, buf, off in ((2, vb, HALO), (1, kb, HALO), (0, qb, 0)):
                for n0 in range(0, HD, qkv_n):
                    cs = _block_matmul(lambda p: _shifted(xa, h0, HS - HM)[_rows(p * HS, HM), :],
                                       lambda p: wqt[_rows((p * 3 + t) * HD, HD), n0:n0 + qkv_n])
                    for qi, val in enumerate(cs):
                        for c in range(qkv_n // 128):
                            buf[(qi % 2) * 4 + n0 // 128 + c, pl.ds(off + (qi // 2) * HM, HM), :] = (
                                val[:, c * 128:(c + 1) * 128])
            for c in range(8):
                row0 = jnp.broadcast_to(vb[c, HALO:HALO + 1, :], (HALO, 128))
                vb[c, :HALO, :] = jnp.where(m == 0, row0, vb[c, :HALO, :])

            gates, seen = [], []
            for n0 in range(0, HD, down_n):
                cs = _block_matmul(
                    lambda p: jnp.concatenate([_shifted(ha, h0, HS - HM)[_rows(j * HS, HM), p * HF:(p + 1) * HF]
                                               for j in range(NC)], axis=1),
                    lambda p: wdt[_rows(p * (F // 2), F // 2), n0:n0 + down_n], seen)
                gates.append([_silu(d) for d in cs])
            _spread([functools.partial(attend, m, h * HM + r, att_rows)
                     for r in range(0, HM, att_rows) for h in range(2)], seen, *att)
            for c in range(4):
                ops = _lhs_ops(ob[c, :HM, :], ob[4 + c, :HM, :], ob[c, HM:, :], ob[4 + c, HM:, :])
                for p in range(7):
                    oa[_rows(p * HM, HM), c * 128:(c + 1) * 128] = ops[p]
            sv = _block_matmul(lambda p: oa[_rows(p * HM, HM), :], lambda p: jnp.concatenate(
                [wot[_rows(p * D + n * HD, HD), :] for n in range(2)], axis=1))
            for qi in range(4):
                rows, cols = pl.ds((qi // 2) * HM, HM), pl.ds((qi % 2) * HD, HD)
                res = xs.at[pl.ds(pl.multiple_of(m * BM, BM), BM)][rows, cols].astype(F32)
                outb.at[slot][rows, cols] = (
                    res + sv[qi] * jnp.concatenate([g[qi] for g in gates], axis=1)).astype(BF16)
            out_copy(m, slot).start()
            return carry

        for c in range(8):
            kb[c, BM:, :] = jnp.zeros((HALO, 128), F32)
            vb[c, BM:, :] = jnp.zeros((HALO, 128), F32)
        with scope('p2'):
            lax.fori_loop(0, NB, scoped('p2_it', block_step), 0)
        with scope('tail'):
            out_copy(NB - 2, 0).wait()
            out_copy(NB - 1, 1).wait()

    def fn(A_x, A_wqkv, A_wo, B_x, B_w_gate, B_w_up, B_w_down):
        any_spec = pl.BlockSpec(memory_space=pl.ANY)
        out = pl.pallas_call(
            kernel,
            in_specs=[any_spec] * 6,
            out_specs=any_spec,
            out_shape=jax.ShapeDtypeStruct((S, D), BF16),
            scratch_shapes=[
                pltpu.VMEM((S, D), BF16),
                pltpu.VMEM((7 * HS // 2, HD), U32),
                pltpu.VMEM((NC * HS // 2, 7 * HF), U32),
                pltpu.VMEM((2, D, FC), BF16),
                pltpu.VMEM((2, D, FC), BF16),
                pltpu.VMEM((2, FC, D), BF16),
                pltpu.VMEM((NQ, 2, 128, D), BF16),
                pltpu.VMEM((2, 2, D, 256), BF16),
                pltpu.VMEM((HD // 2, 7 * HF), U32),
                pltpu.VMEM((HD // 2, 7 * HF), U32),
                pltpu.VMEM((7 * F // 4, HD), U32),
                pltpu.VMEM((21 * HD // 2, HD), U32),
                pltpu.VMEM((7 * HD, 256), U32),
                pltpu.VMEM((8, BM, 128), F32),
                pltpu.VMEM((8, HALO + BM, 128), F32),
                pltpu.VMEM((8, HALO + BM, 128), F32),
                pltpu.VMEM((8, BM, 128), F32),
                pltpu.VMEM((7 * HM // 2, HD), U32),
                pltpu.VMEM((2, BM, D), BF16),
                pltpu.SemaphoreType.DMA((NB,)),
                pltpu.SemaphoreType.DMA((5, 2)),
                pltpu.SemaphoreType.DMA((2, 2)),
                pltpu.SemaphoreType.DMA((2,)),
            ],
            compiler_params=pltpu.CompilerParams(vmem_limit_bytes=120 * 2**20, flags=flags,
                                                 disable_bounds_checks=nobc, disable_semaphore_checks=nosc),
        )(A_x.reshape(S, D), A_wqkv, A_wo, B_w_gate, B_w_up, B_w_down)
        return out.reshape(1, S, D)

    return fn


@jax.jit
def pallas_recurrent_scan__sliding_local_dilated__geglu_ffn__prompt_kernel(
        A_x, A_wqkv, A_wo, B_x, B_w_gate, B_w_up, B_w_down):
    return make(nobc=True,ln=(-0.1,0.75),att=(-0.03,0.6),side=(0.05,0.9))(A_x, A_wqkv, A_wo, B_x, B_w_gate, B_w_up, B_w_down)
```

```python
import contextlib
import functools
import numpy as np
import jax
import jax.numpy as jnp
from jax import lax
from jax.experimental import pallas as pl
from jax.experimental.pallas import tpu as pltpu

S, D, F = 2048, 1024, 3584
DH, WIN, DIL = 32, 8, 2
BM = 256
HM, QM = BM // 2, BM // 4
NB = S // BM
FC = 512
NC = F // FC
HD, QD = D // 2, D // 4
QS, QF = S // 4, F // 4
XR = (NB + 1) * QM
HALO = 16
EV = {"XLA_TPU_EVENLY_DISTRIBUTE_CRITICAL_NODES": True}
F32, BF16, U32 = jnp.float32, jnp.bfloat16, jnp.uint32
ORDER = (1, 2, 0, 3, 5, 4, 6)
SKEW = (1.0, 0.5, 2.0, 1.0)
LHS_GROUPS = ((1, 2), (0, 3, 5), (4, 6))
RHS_GROUPS = ((1, 2), (3, 5), (0, 4, 6))


def _pack(v):
    return pltpu.bitcast(v.astype(BF16), U32)


def _unpack(v):
    return pltpu.bitcast(v, BF16)


def _rows(start, n):
    return pl.ds(start // 2, n // 2)


def _shifted(ref, rows, limit):
    start = rows // 2 if isinstance(rows, int) else pl.multiple_of(rows >> 1, 8)
    return ref.at[pl.ds(start, ref.shape[0] - limit // 2)]


def _scaled(v, s):
    return v if s == 1.0 else v * np.float32(s)


def _lhs_ops(a):
    t, e = a[0] + a[3], a[1] + a[2]
    return [t, a[0] - a[1], a[0] + a[1], t - e, a[3] - a[1], t + e, a[3] + a[1]]


def _rhs_ops(b):
    t, e = b[0] + b[3], b[1] + b[2]
    return [t + t, b[3] - b[1], b[3] + b[1], b[0] + b[1], t + e, b[0] - b[1], t - e]


def _combine(m):
    base, d = m[0] - (m[1] + m[2]), m[2] - m[1]
    return [(base - m[4]) - m[6], d, (((d - m[3]) + m[5]) + m[4]) - m[6], (base - m[3]) - m[5]]


def _paced(ops, quads, pace):
    hold = pace()
    return ops([quads[0], hold(quads[1]), quads[2], quads[3]])


def _two_level(ops, group, blk, pace, pace_outer):
    outer = [_paced(ops, [blk(a, b) for a in range(4)], pace_outer) for b in range(4)]
    return [(7 * p + q, o) for p in group for q, o in enumerate(_paced(ops, [outer[b][p] for b in range(4)], pace))]


def _place(a, b):
    return (a // 2) * 2 + b // 2, (a % 2) * 2 + b % 2


def _matmul1(lhs, rhs, seen, base=0):
    m = [None] * 7
    for p in ORDER:
        m[p] = jnp.dot(lhs(base + p), rhs(base + p), preferred_element_type=F32)
        seen.append(m[p])
    return _combine(m)


def _matmul2(lhs, rhs, seen):
    m = [None] * 7
    for p in ORDER:
        m[p] = _matmul1(lhs, rhs, seen, 7 * p)
    out = [_combine([m[p][b] for p in range(7)]) for b in range(4)]
    return {(a, b): out[b][a] for a in range(4) for b in range(4)}


def _geglu(g, u, s, out):
    c = np.sqrt(2.0 / np.pi)
    t = jnp.tanh(g * (np.float32(c / s) + np.float32(c * 0.044715 / s ** 3) * (g * g)))
    return ((np.float32(0.5 * out / s ** 2) * g) * (1.0 + t)) * u


def _silu(d, s, out):
    return (np.float32(0.5 * out / s) * d) * (1.0 + jnp.tanh(np.float32(0.5 / s) * d))


def _permute_columns(cols, pace):
    lane = lax.broadcasted_iota(jnp.int32, cols[0].shape, 1)
    cols = list(cols)
    for t in range(3):
        s = 4 << t
        low = (lane & s) == 0
        for c in range(len(cols)):
            if c & (1 << t):
                continue
            hold = pace()
            a, b = hold(cols[c]), hold(cols[c | (1 << t)])
            cols[c] = jnp.where(low, a, pltpu.roll(b, s, 1))
            cols[c | (1 << t)] = jnp.where(low, pltpu.roll(a, 128 - s, 1), b)
    return cols


def _pacer(products, count, lo, hi):
    tiles = [(m, r, c) for m in products for c in range(0, m.shape[1], 128 if m.shape[1] > 256 else 256)
             for r in range(0, m.shape[0], 8)]
    calls = [0]

    def pace():
        k = int(np.floor((lo + (hi - lo) * calls[0] / count) * len(tiles)))
        calls[0] += 1
        assert calls[0] <= count, count
        if k < 0:
            return _now()
        m, r, c = tiles[k]
        tile = m[r:r + 8, c:c + 128]

        def hold(v):
            never = jnp.tile(tile, (v.shape[0] // 8, v.shape[1] // 128)) > np.float32(np.inf)
            return jnp.where(never, jnp.zeros_like(v), v)
        return hold
    return pace


def _now():
    return lambda v: v


def make(scopes=False, att_rows=8, qkv_n=512, flags=None, nobc=True, nosc=False, att=(-0.03, 0.7),
         side=(0.0, 0.97), ln0=(-0.05, 0.45), ln=(0.4, 0.97), ln_lag=4, hop=(-0.02, 0.98), gate_q=True, po=True):
    scope = jax.named_scope if scopes else (lambda n: contextlib.nullcontext())
    steps = 19 if po else 7

    def scoped(name, f):
        def g(*a):
            with scope(name):
                return f(*a)
        return g

    def kernel(x_hbm, wqkv_hbm, wo_hbm, wg_hbm, wu_hbm, wd_hbm, out_hbm,
               xs, xa1, xa2, hs, wt0, wt1, wdt, wqt, wot, wg_s, wu_s, wd_s, wq_s, wo_s, kb, vb,
               sem_x, sem_w, sem_a, sem_o):
        wt, st, outb = (wt0, wt1), kb, wq_s.at[0]

        def x_copy(m):
            rows = pl.ds(pl.multiple_of(m * BM, BM), BM)
            return pltpu.make_async_copy(x_hbm.at[rows], xs.at[rows], sem_x.at[m])

        def w_copies(j, slot):
            col = pl.ds(pl.multiple_of(j * FC, FC), FC)
            return (pltpu.make_async_copy(wg_hbm.at[:, col], wg_s.at[slot], sem_w.at[0, slot]),
                    pltpu.make_async_copy(wu_hbm.at[:, col], wu_s.at[slot], sem_w.at[1, slot]))

        def side_copies(i, slot):
            cols = pl.ds(pl.multiple_of((i >> 1) * D, D), D)
            out = [pltpu.make_async_copy(
                wqkv_hbm.at[pl.ds(pl.multiple_of(h * HD + (i & 1) * QD, QD), QD), cols],
                wq_s.at[slot, h], sem_w.at[2 + h, slot]) for h in range(2)]
            return out + [pltpu.make_async_copy(wd_hbm.at[pl.ds(pl.multiple_of((i + 1) * FC, FC), FC)],
                                                wd_s.at[slot], sem_w.at[4, slot])]

        def once_copies():
            return [pltpu.make_async_copy(wo_hbm.at[:, pl.ds(h * HD + n * 256, 256)], wo_s.at[n, h],
                                          sem_a.at[2 * n + h]) for n in range(2) for h in range(2)] + [
                pltpu.make_async_copy(wd_hbm.at[:FC], wd_s.at[2], sem_a.at[4])]

        def layernorm(src, dst1, dst2, pace_stats, pace, skip=0):
            mean = {}
            groups = [k * QM + r for r in range(0, QM, 16) for k in range(4)]
            for n in range(len(groups) + ln_lag):
                if n < len(groups):
                    r = groups[n]
                    x = src[r:r + 16, :].astype(F32)
                    x = jnp.concatenate([pace_stats()(x[:, :128]), x[:, 128:]], axis=1)
                    mean[r] = jnp.broadcast_to(jnp.mean(x, axis=-1, keepdims=True), (16, 128))
                    st[0, r:r + 16, :] = mean[r]
                if n >= ln_lag:
                    r = groups[n - ln_lag]
                    xc = src[r:r + 16, :].astype(F32) - jnp.tile(pace_stats()(mean[r]), (1, 8))
                    st[1, r:r + 16, :] = jnp.broadcast_to(
                        lax.rsqrt(jnp.mean(xc * xc, axis=-1, keepdims=True) + 1e-5), (16, 128))
            for r in range(0, QM, 16):
                for c in (0, 128):
                    one = []
                    for b in range(4):
                        hold, quads = pace(), []
                        for a in range(4):
                            rq, cq = _place(a, b)
                            rows = slice(rq * QM + r, rq * QM + r + 16)
                            x = src[rows, cq * QD + c:cq * QD + c + 128].astype(F32)
                            quads.append((x - hold(st[0, rows, :])) * _scaled(st[1, rows, :], SKEW[a]))
                        one.append(_lhs_ops(quads))
                        for p in range(7):
                            col = (b % 2) * QD + c
                            dst1[_rows(p * 2 * XR + (b // 2) * QM + r, 16), col:col + 128] = _pack(one[b][p])
                    for p in range(7):
                        two = _paced(_lhs_ops, [_scaled(one[b][p], SKEW[b]) for b in range(4)], pace)
                        for q in range(7):
                            dst2[_rows((7 * p + q) * XR + skip + r, 16), c:c + 128] = _pack(two[q])

        def prep_two(src, dst, r, c, height, width, stride, col, pace):
            def blk(a, b):
                rq, cq = _place(a, b)
                v = src[rq * height + r:rq * height + r + 16, cq * width + c:cq * width + c + 128]
                return _scaled(v.astype(F32), SKEW[a] * SKEW[b])
            for group in RHS_GROUPS:
                for n, op in _two_level(_rhs_ops, group, blk, pace, pace if po else _now):
                    dst[_rows(n * stride + r, 16), col:col + 128] = _pack(op)

        def prep_chunk(k, slot, r0, limit, r, pace):
            prep_two((wg_s, wu_s)[k].at[slot, pl.ds(r0, D - limit)], _shifted(wt[slot], r0, limit),
                     r, 0, QD, 128, QD, k * 128, pace)

        def prep_down(slot, chunk, r0, limit, r, c, pace):
            prep_two(wd_s.at[slot, pl.ds(r0, FC - limit)], _shifted(wdt, chunk * 128 + r0, (NC - 1) * 128 + limit),
                     r, c, 128, QD, QF, c, pace)

        def gate_up(src, rhs, dst, r0, side_work):
            out = []
            for k in range(2):
                seen = []
                out.append(_matmul2(lambda p: _unpack(src[_rows(p * XR + r0, QM), :]),
                                    lambda p: _unpack(rhs[_rows(p * QD, QD), k * 128:(k + 1) * 128]), seen))
                side_work(k, seen)
            for a, b in out[0]:
                s = SKEW[a] * SKEW[b]
                dst[r0:r0 + QM, (4 * a + b) * 128:(4 * a + b + 1) * 128] = _geglu(
                    out[0][a, b], out[1][a, b], 4 * s, s)

        def prep_qkv(i, slot, half, r, pace):
            src = wq_s.at[slot, :, pl.ds(pl.multiple_of(half * 128, 128), 128)]
            cols = _permute_columns([pltpu.bitcast(src[h, r:r + 16, c * 128:(c + 1) * 128], U32)
                                     for h in range(2) for c in range(8)], pace if gate_q else _now)
            for c in range(4):
                quads = [_scaled(_unpack(cols[4 * a + c]).astype(F32), SKEW[a]) for a in range(4)]
                for p, op in enumerate(_paced(_rhs_ops, quads, pace)):
                    _shifted(wqt, i * QD + half * 128, 5 * QD + 128)[
                        _rows(p * 3 * HD + r, 16), c * 128:(c + 1) * 128] = _pack(op)

        def prep_wo(i, c0, g2, e2, pace):
            n, r0 = i >> 2, pl.multiple_of((i & 3) * 32, 32)
            low = lax.broadcasted_iota(jnp.int32, (8, 128), 0) < 4
            src = wo_s.at[n, :, pl.ds(r0, D - 96)]
            new = {}
            for h in range(2):
                hold = pace()
                for e in (e2, e2 + 2):
                    t = [hold(src[h, pl.ds((4 * g2 + c) * 128 + e * 8, 8), c0:c0 + 128].astype(F32))
                         for c in range(4)]
                    new[h, 2 * e] = jnp.concatenate(
                        [jnp.where(low, t[c], pltpu.roll(t[c + 1], 4, 0)) for c in (0, 2)], axis=0)
                    new[h, 2 * e + 1] = jnp.concatenate(
                        [jnp.where(low, pltpu.roll(t[c], 4, 0), t[c + 1]) for c in (0, 2)], axis=0)
            for e in (2 * e2, 2 * e2 + 1):
                quads = (new[0, e], new[1, e], new[0, e + 4], new[1, e + 4])
                for p, op in enumerate(_paced(_rhs_ops, [_scaled(v, s) for v, s in zip(quads, SKEW)], pace)):
                    _shifted(wot, n * HD + r0, HD + 96)[
                        _rows(p * D + e * 128 + 16 * g2, 16), c0:c0 + 128] = _pack(op)

        first = w_copies(0, 0)
        first[0].start()
        x_copy(0).start()
        with scope('w_g'):
            first[0].wait()
        first[1].start()
        for r in range(0, QD, 16):
            prep_chunk(0, 0, 0, 0, r, _now)
        with scope('w_x'):
            x_copy(0).wait()
        x_copy(1).start()
        layernorm(xs, xa1, xa2, _now, _now)
        with scope('w_u'):
            first[1].wait()
        for c in piece_copies(wg_hbm, wu_hbm, wg_s, wu_s, sem_w, 0):
            c.start()
        x_copy(2).start()
        for r in range(0, QD, 16):
            prep_chunk(1, 0, 0, 0, r, _now)

        def first_step(m, carry):
            for c in piece_copies(wg_hbm, wu_hbm, wg_s, wu_s, sem_w, m):
                c.wait()

            @pl.when(m + 1 < NB)
            def _():
                x_copy(m + 1).wait()
                for c in piece_copies(wg_hbm, wu_hbm, wg_s, wu_s, sem_w, m + 1):
                    c.start()

            @pl.when(m + 3 < NB)
            def _():
                x_copy(m + 3).start()

            later = [*w_copies(2, 0), *side_copies(0, 1), *once_copies()]
            for at, n in enumerate(((0,), (1,), (2, 3), (4,), (5, 6), (7, 8), (9,))):
                @pl.when(m == at)
                def _():
                    for i in n:
                        later[i].start()

            rows = _shifted(xa2, m * QM, (NB - 1) * QM)
            nxt = xs.at[pl.ds(pl.multiple_of(jnp.minimum(m + 1, NB - 1) * BM, BM), BM)]
            dst1 = _shifted(xa1, (m + 1) * HM, NB * HM)

            def side_work(k, seen):
                if k == 0:
                    pace = _pacer(seen, 4 * steps, *side)
                    for i in range(4):
                        prep_chunk(i // 2, 1, pl.multiple_of(m * 32, 32), 224, (i % 2) * 16, pace)
                every.extend(seen)

            every = []
            gate_up(rows, wt[0], hs.at[pl.ds(pl.multiple_of(m * QM, QM), QM)], 0, side_work)
            layernorm(nxt, dst1, rows, _pacer(every, 32, *ln0), _pacer(every, 88, *ln), QM)
            return carry

        with scope('p0'):
            lax.fori_loop(0, NB, scoped('p0_it', first_step), 0)
        with scope('w_end'):
            for c in once_copies():
                c.wait()

        def half_step(j, slot, half, carry):
            i8 = jnp.minimum(2 * (j - 1) + half, 7)
            src = _shifted(xa2, half * (QS // 2), QS // 2)
            dst = hs.at[pl.ds(pl.multiple_of(j * QS + half * (QS // 2), QS // 2), QS // 2)]

            def side_work(n, k, seen):
                r = 2 * n + k
                extra = r % 4 == 0
                prep_qkv(j - 1, slot, half, r * 16, _pacer(seen, 28 if gate_q else 4, *side))
                pace = _pacer(seen, (4 if extra else 3) * steps + 4, *side)
                prep_wo(i8, (r // 4) * 128, (r // 2) % 2, r % 2, pace)
                prep_down(slot, j, pl.multiple_of(half * 64, 64), 64, (r // 2) * 16, (r % 2) * 128, pace)
                for t in range(2):
                    prep_chunk(t, 1 - slot, pl.multiple_of(half * 128, 128), 128, r * 16, pace)
                if extra:
                    prep_down(2, 0, pl.multiple_of(i8 * 16, 16), 112, 0, (r // 4) * 128, pace)

            for n in range(4):
                gate_up(src, wt[slot], dst, n * QM, functools.partial(side_work, n))
            return carry

        def pair_step(i, carry):
            for slot in (1, 0):
                j = 2 * i + 2 - slot
                for c in side_copies(j - 1, slot):
                    c.wait()

                @pl.when(j + 1 < NC)
                def _():
                    for c in w_copies(j + 1, 1 - slot):
                        c.wait()
                    for c in side_copies(j, 1 - slot):
                        c.start()

                @pl.when(j + 2 < NC)
                def _():
                    for c in w_copies(j + 2, slot):
                        c.start()

                lax.fori_loop(0, 2, scoped('p1_it', functools.partial(half_step, j, slot)), 0)
            return carry

        with scope('p1'):
            lax.fori_loop(0, NC // 2, pair_step, 0)

        def out_copy(m, slot):
            return pltpu.make_async_copy(outb.at[slot], out_hbm.at[pl.ds(pl.multiple_of(m * BM, BM), BM)],
                                         sem_o.at[slot])

        def attend(m, q, r0, n, hold):
            lane = lax.broadcasted_iota(jnp.int32, (n, 128), 1)
            logits = []
            q = [hold(t) for t in q]
            for w in range(WIN):
                acc = None
                for c in (4, 5, 6, 7, 0, 1, 2, 3):
                    t = q[c] * kb[c, pl.ds(HALO + r0 - DIL * w, n), :]
                    acc = t if acc is None else acc + t
                for s in (1, 2):
                    acc = acc + jnp.take_along_axis(acc, lane ^ s, axis=1)
                acc = acc * np.float32(DH ** -0.5)
                if r0 < DIL * w:
                    pos = m * BM + r0 + lax.broadcasted_iota(jnp.int32, (n, 128), 0)
                    acc = jnp.where(pos >= DIL * w, acc, np.float32(-1e9))
                logits.append(acc)
            mx = functools.reduce(jnp.maximum, logits)
            e = [jnp.exp(l - mx) for l in logits]
            inv = 1.0 / functools.reduce(lambda a, b: a + b, e)
            pr = [t * inv for t in e]
            out = []
            for c in range(8):
                acc = None
                for w in range(WIN):
                    t = pr[w] * vb[c, pl.ds(HALO + r0 - DIL * w, n), :]
                    acc = t if acc is None else acc + t
                out.append(acc)
            return out

        def block_step(m, carry):
            slot = m & 1

            @pl.when(m >= 2)
            def _():
                out_copy(m - 2, slot).wait()

            for c in range(8):
                kb[c, :HALO, :] = kb[c, BM:, :]
                vb[c, :HALO, :] = vb[c, BM:, :]
            early, q = [], {}
            for t, buf in ((2, vb), (1, kb), (0, None)):
                for n0 in range(0, HD, qkv_n):
                    cs = _matmul1(lambda p: _unpack(_shifted(xa1, m * HM, NB * HM)[_rows(p * 2 * XR, HM), :]),
                                  lambda p: _unpack(wqt[_rows((p * 3 + t) * HD, HD), n0:n0 + qkv_n]), early)
                    for a, val in enumerate(cs):
                        val = _scaled(val, 0.5 / SKEW[a])
                        for c in range(qkv_n // 128):
                            col, tile = (a % 2) * 4 + n0 // 128 + c, val[:, c * 128:(c + 1) * 128]
                            if buf is None:
                                q[a // 2, col] = tile
                            else:
                                buf[col, pl.ds(HALO + (a // 2) * HM, HM), :] = tile
            for c in range(8):
                row0 = jnp.broadcast_to(vb[c, HALO:HALO + 1, :], (HALO, 128))
                vb[c, :HALO, :] = jnp.where(m == 0, row0, vb[c, :HALO, :])

            hv = hs.at[pl.ds(pl.multiple_of(m * QM, QM), NC * QS - (NB - 1) * QM)]
            pace, ha = _pacer(early, 28 * steps, *hop), {}
            for group in LHS_GROUPS:
                for j in range(NC):
                    for r in range(0, QM, 16):
                        blk = lambda a, b: hv[j * QS + r:j * QS + r + 16, (4 * a + b) * 128:(4 * a + b + 1) * 128]
                        for n, op in _two_level(_lhs_ops, group, blk, pace, pace if po else _now):
                            ha[n, j, r] = op.astype(BF16)
            seen = []
            down = _matmul2(
                lambda p: jnp.concatenate([jnp.concatenate([ha[p, j, r] for j in range(NC)], axis=1)
                                           for r in range(0, QM, 16)], axis=0),
                lambda p: _unpack(wdt[_rows(p * QF, QF), :]), seen)
            pace, o = _pacer(seen, BM // att_rows, *att), {}
            for r in range(0, HM, att_rows):
                for h in range(2):
                    o[h, r] = attend(m, [q[h, c][r:r + att_rows] for c in range(8)], h * HM + r, att_rows, pace())
            oa = _lhs_ops([_scaled(jnp.concatenate(
                [jnp.concatenate(o[a // 2, r][4 * (a % 2):4 * (a % 2) + 4], axis=1)
                 for r in range(0, HM, att_rows)], axis=0), SKEW[a]) for a in range(4)])
            sv = _matmul1(lambda p: oa[p].astype(BF16), lambda p: _unpack(jnp.concatenate(
                [wot[_rows(p * D + n * HD, HD), :] for n in range(2)], axis=1)), [])
            for (a, b), d in down.items():
                rq, cq = _place(a, b)
                rows, cols = pl.ds(rq * QM, QM), pl.ds(cq * QD, QD)
                res = xs.at[pl.ds(pl.multiple_of(m * BM, BM), BM)][rows, cols].astype(F32)
                att_out = sv[a][(b // 2) * QM:(b // 2 + 1) * QM, (b % 2) * QD:(b % 2 + 1) * QD]
                gate = _silu(d, 4 * SKEW[a] * SKEW[b], 0.5 / SKEW[a])
                outb.at[slot][rows, cols] = (res + att_out * gate).astype(BF16)
            out_copy(m, slot).start()
            return carry

        for c in range(8):
            kb[c, BM:, :] = jnp.zeros((HALO, 128), F32)
            vb[c, BM:, :] = jnp.zeros((HALO, 128), F32)
        with scope('p2'):
            lax.fori_loop(0, NB, scoped('p2_it', block_step), 0)
        with scope('tail'):
            out_copy(NB - 2, 0).wait()
            out_copy(NB - 1, 1).wait()

    def piece_copies(wg_hbm, wu_hbm, wg_s, wu_s, sem_w, m):
        out = []
        for k, (src, dst) in enumerate(((wg_hbm, wg_s), (wu_hbm, wu_s))):
            for q in range(4):
                rows = pl.ds(pl.multiple_of(q * QD + m * 32, 32), 32)
                out.append(pltpu.make_async_copy(src.at[rows, FC:2 * FC], dst.at[1, rows], sem_w.at[k, 1]))
        return out

    def fn(A_x, A_wqkv, A_wo, B_x, B_w_gate, B_w_up, B_w_down):
        any_spec = pl.BlockSpec(memory_space=pl.ANY)
        out = pl.pallas_call(
            kernel,
            in_specs=[any_spec] * 6,
            out_specs=any_spec,
            out_shape=jax.ShapeDtypeStruct((S, D), BF16),
            scratch_shapes=[
                pltpu.VMEM((S, D), BF16),
                pltpu.VMEM((7 * XR, HD), U32),
                pltpu.VMEM((49 * XR // 2, QD), U32),
                pltpu.VMEM((NC * QS, 16 * 128), F32),
                pltpu.VMEM((49 * QD // 2, 256), U32),
                pltpu.VMEM((49 * QD // 2, 256), U32),
                pltpu.VMEM((49 * QF // 2, QD), U32),
                pltpu.VMEM((21 * HD // 2, HD), U32),
                pltpu.VMEM((7 * HD, 256), U32),
                pltpu.VMEM((2, D, FC), BF16),
                pltpu.VMEM((2, D, FC), BF16),
                pltpu.VMEM((3, FC, D), BF16),
                pltpu.VMEM((2, 2, QD, D), BF16),
                pltpu.VMEM((2, 2, D, 256), BF16),
                pltpu.VMEM((8, HALO + BM, 128), F32),
                pltpu.VMEM((8, HALO + BM, 128), F32),
                pltpu.SemaphoreType.DMA((NB,)),
                pltpu.SemaphoreType.DMA((5, 2)),
                pltpu.SemaphoreType.DMA((5,)),
                pltpu.SemaphoreType.DMA((2,)),
            ],
            compiler_params=pltpu.CompilerParams(vmem_limit_bytes=126 * 2**20, flags=flags,
                                                 disable_bounds_checks=nobc, disable_semaphore_checks=nosc),
        )(A_x.reshape(S, D), A_wqkv, A_wo, B_w_gate, B_w_up, B_w_down)
        return out.reshape(1, S, D)

    return fn


@jax.jit
def pallas_recurrent_scan__sliding_local_dilated__geglu_ffn__prompt_kernel(
        A_x, A_wqkv, A_wo, B_x, B_w_gate, B_w_up, B_w_down):
    return make(po=False)(A_x, A_wqkv, A_wo, B_x, B_w_gate, B_w_up, B_w_down)
```

```python
import contextlib
import functools
import numpy as np
import jax
import jax.numpy as jnp
from jax import lax
from jax.experimental import pallas as pl
from jax.experimental.pallas import tpu as pltpu

S, D, F = 2048, 1024, 3584
DH, WIN, DIL = 32, 8, 2
BM = 256
NB = S // BM
HALO = 16
EV = {"XLA_TPU_EVENLY_DISTRIBUTE_CRITICAL_NODES": True}
F32, BF16, U32 = jnp.float32, jnp.bfloat16, jnp.uint32


def _pack(v):
    return pltpu.bitcast(v.astype(BF16), U32)


def _unpack(v):
    return pltpu.bitcast(v, BF16)


def _rows(start, n):
    return pl.ds(start // 2, n // 2)


def _shifted(ref, rows, limit):
    start = rows // 2 if isinstance(rows, int) else pl.multiple_of(rows >> 1, 8)
    return ref.at[pl.ds(start, ref.shape[0] - limit // 2)]


def _dot(a, b):
    return jnp.dot(a, b, preferred_element_type=F32)


def _geglu(g, u):
    c = np.sqrt(2.0 / np.pi)
    t = jnp.tanh(g * (np.float32(c) + np.float32(c * 0.044715) * (g * g)))
    return ((0.5 * g) * (1.0 + t)) * u


def _permute_columns(cols, pace):
    lane = lax.broadcasted_iota(jnp.int32, cols[0].shape, 1)
    hold = pace()
    cols = [hold(c) for c in cols]
    for t in range(3):
        s = 4 << t
        low = (lane & s) == 0
        for c in range(8):
            if c & (1 << t):
                continue
            a, b = cols[c], cols[c | (1 << t)]
            cols[c] = jnp.where(low, a, pltpu.roll(b, s, 1))
            cols[c | (1 << t)] = jnp.where(low, pltpu.roll(a, 128 - s, 1), b)
    return cols


def _pacer(products, count, lo, hi):
    tiles = [(m, r, c) for m in products for c in range(0, m.shape[1], 128) for r in range(0, m.shape[0], 8)]
    calls = [0]

    def pace():
        k = int(np.floor((lo + (hi - lo) * calls[0] / count) * len(tiles)))
        calls[0] += 1
        assert calls[0] <= count, count
        if k < 0:
            return _now()
        m, r, c = tiles[k]
        tile = m[r:r + 8, c:c + 128]

        def hold(v):
            never = jnp.tile(tile, (v.shape[0] // 8, v.shape[1] // 128)) > np.float32(np.inf)
            return jnp.where(never, jnp.zeros_like(v), v)
        return hold
    return pace


def _now():
    return lambda v: v


def make(scopes=False, F0=256, FC=256, sub=256, att_rows=8, kd=512, flags=None, nobc=True, nosc=False,
         att=(-0.03, 0.7), side=(0.0, 0.9), ln=(-0.1, 0.7), ln_lag=4):
    scope = jax.named_scope if scopes else (lambda n: contextlib.nullcontext())
    NC = (F - F0) // FC
    assert F0 + NC * FC == F and NC >= 8

    def scoped(name, f):
        def g(*a):
            with scope(name):
                return f(*a)
        return g

    def kernel(x_hbm, wqkv_hbm, wo_hbm, wg_hbm, wu_hbm, wd_hbm, out_hbm,
               xs, xn, hs, wqt, wot, wg_s, wu_s, wd_s, wq_s, wo_s, kb, vb, outb,
               sem_x, sem_w, sem_a, sem_o):
        st = kb

        def x_copy(m):
            rows = pl.ds(m * BM, BM)
            return pltpu.make_async_copy(x_hbm.at[rows], xs.at[rows], sem_x.at[m])

        def w_copies(j, slot):
            col = pl.ds(pl.multiple_of(F0 + j * FC, 128), FC)
            return (pltpu.make_async_copy(wg_hbm.at[:, col], wg_s.at[slot], sem_w.at[0, slot]),
                    pltpu.make_async_copy(wu_hbm.at[:, col], wu_s.at[slot], sem_w.at[1, slot]))

        def wq_copy(i):
            rows = pl.ds(pl.multiple_of(i * 128, 128), 128)
            return pltpu.make_async_copy(wqkv_hbm.at[rows], wq_s.at[rows], sem_w.at[2, i & 1])

        def wo_copy(n):
            return pltpu.make_async_copy(wo_hbm.at[:, n * 512:(n + 1) * 512], wo_s.at[n], sem_a.at[n])

        def wd_copy():
            return pltpu.make_async_copy(wd_hbm, wd_s, sem_a.at[2])

        def layernorm(blocks, pace):
            groups = [m * BM + r for m in blocks for r in range(0, BM, 16)]
            mean, rstd = {}, {}
            for n in range(len(groups) + 2 * ln_lag):
                if n < len(groups):
                    r = groups[n]
                    x = xs[r:r + 16, :].astype(F32)
                    x = jnp.concatenate([pace()(x[:, :128]), x[:, 128:]], axis=1)
                    mean[r] = jnp.broadcast_to(jnp.mean(x, axis=-1, keepdims=True), (16, 128))
                    st[0, r % BM:r % BM + 16, :] = mean[r]
                if 0 <= n - ln_lag < len(groups):
                    r = groups[n - ln_lag]
                    xc = xs[r:r + 16, :].astype(F32) - jnp.tile(pace()(mean[r]), (1, 8))
                    rstd[r] = lax.rsqrt(jnp.mean(xc * xc, axis=-1, keepdims=True) + 1e-5)
                    st[1, r % BM:r % BM + 16, :] = jnp.broadcast_to(rstd[r], (16, 128))
                if 0 <= n - 2 * ln_lag:
                    r = groups[n - 2 * ln_lag]
                    xc = xs[r:r + 16, :].astype(F32) - jnp.tile(pace()(mean[r]), (1, 8))
                    xn[_rows(r, 16), :] = _pack(xc * rstd[r])

        def gate_up(dst, slot, r0, n, width, mid=None):
            seen = []
            if mid is not None:
                g = _dot(_unpack(xn[_rows(r0, n), :]), wg_s.at[slot][:, :width])
                mid()
                u = _dot(_unpack(xn[_rows(r0, n), :]), wu_s.at[slot][:, :width])
                dst[_rows(r0, n), :width] = _pack(_geglu(g, u))
                return [u]
            for c in range(0, width, 128):
                g = _dot(_unpack(xn[_rows(r0, n), :]), wg_s.at[slot][:, c:c + 128])
                u = _dot(_unpack(xn[_rows(r0, n), :]), wu_s.at[slot][:, c:c + 128])
                dst[_rows(r0, n), c:c + 128] = _pack(_geglu(g, u))
                seen += [g, u]
            return seen

        def prep_qkv(i, t, r, pace):
            src = wq_s.at[pl.ds(pl.multiple_of(i * 128, 128), 128)]
            cols = _permute_columns([pltpu.bitcast(src[r:r + 16, t * D + c * 128:t * D + (c + 1) * 128], U32)
                                     for c in range(8)], pace)
            _shifted(wqt, i * 128, D - 128)[_rows(r, 16), t * D:(t + 1) * D] = jnp.concatenate(cols, axis=1)

        def prep_wo(i, g2, e, pace):
            n, r0 = i >> 2, pl.multiple_of((i & 3) * 32, 32)
            low = lax.broadcasted_iota(jnp.int32, (8, 512), 0) < 4
            src, hold = wo_s.at[n, pl.ds(r0, D - 96)], pace()
            t = [hold(src[pl.ds((4 * g2 + c) * 128 + e * 8, 8), :].astype(F32)) for c in range(4)]
            dst = _shifted(wot, n * D + r0, D + 96)
            dst[_rows(2 * e * 128 + 16 * g2, 16), :] = _pack(jnp.concatenate(
                [jnp.where(low, t[c], pltpu.roll(t[c + 1], 4, 0)) for c in (0, 2)], axis=0))
            dst[_rows((2 * e + 1) * 128 + 16 * g2, 16), :] = _pack(jnp.concatenate(
                [jnp.where(low, pltpu.roll(t[c], 4, 0), t[c + 1]) for c in (0, 2)], axis=0))

        first = [pltpu.make_async_copy(src.at[:, :F0], dst.at[1, :, :F0], sem_w.at[k, 1])
                 for k, (src, dst) in enumerate(((wg_hbm, wg_s), (wu_hbm, wu_s)))]
        h0 = _shifted(hs, NC * S, NC * S)
        x_copy(0).start()
        x_copy(1).start()
        with scope('w_x0'):
            x_copy(0).wait()
        first[0].start()
        layernorm([0], _now)
        with scope('w_x1'):
            x_copy(1).wait()
        first[1].start()
        x_copy(2).start()
        layernorm([1], _now)
        with scope('w_g'):
            first[0].wait()
        x_copy(3).start()

        def arrive():
            with scope('w_u'):
                first[1].wait()
                x_copy(2).wait()
            x_copy(4).start()
            x_copy(5).start()

        seen = gate_up(h0, 1, 0, 2 * BM, F0, arrive)
        layernorm([2], _pacer(seen, 48, *ln))
        for now, nxt, start in (((2,), (3, 4), lambda: [x_copy(6), x_copy(7)]),
                                ((3, 4), (5, 6, 7), lambda: [*w_copies(0, 0)]),
                                ((5, 6, 7), (), lambda: [wq_copy(0), wo_copy(0)])):
            with scope('w_p0'):
                for m in nxt:
                    x_copy(m).wait()
            for c in start():
                c.start()
            seen = [p for m in now for p in gate_up(h0, 1, m * BM, BM, F0)]
            layernorm(nxt, _pacer(seen, 48 * len(nxt), *ln))
        with scope('w_end'):
            wo_copy(0).wait()

        def chunk_step(j, carry):
            slot = j & 1
            for c in w_copies(j, slot):
                c.wait()

            @pl.when(j < 8)
            def _():
                wq_copy(j).wait()

            @pl.when(j == 4)
            def _():
                wo_copy(1).wait()

            @pl.when(j + 1 < NC)
            def _():
                for c in w_copies(j + 1, 1 - slot):
                    c.start()

            @pl.when(j + 1 < 8)
            def _():
                wq_copy(j + 1).start()

            @pl.when(j == 3)
            def _():
                wo_copy(1).start()

            @pl.when(j == NC - 2)
            def _():
                wd_copy().start()

            i = jnp.minimum(j, 7)
            seen = [p for r0 in range(0, S, sub) for p in gate_up(_shifted(hs, j * S, NC * S), slot, r0, sub, FC)]
            pace = _pacer(seen, 32, *side)
            for r in range(8):
                for t in range(3):
                    prep_qkv(i, t, r * 16, pace)
                prep_wo(i, r // 4, r % 4, pace)
            return carry

        with scope('p1'):
            lax.fori_loop(0, NC, scoped('p1_it', chunk_step), 0)
        wd_copy().wait()

        def out_copy(m, slot):
            return pltpu.make_async_copy(outb.at[slot], out_hbm.at[pl.ds(pl.multiple_of(m * BM, BM), BM)],
                                         sem_o.at[slot])

        def attend(m, q, r0, n, hold):
            lane = lax.broadcasted_iota(jnp.int32, (n, 128), 1)
            q = [hold(q[:, c * 128:(c + 1) * 128]) for c in range(8)]
            logits = []
            for w in range(WIN):
                acc = None
                for c in range(8):
                    t = q[c] * kb[c, pl.ds(HALO + r0 - DIL * w, n), :]
                    acc = t if acc is None else acc + t
                for s in (1, 2):
                    acc = acc + jnp.take_along_axis(acc, lane ^ s, axis=1)
                acc = acc * np.float32(DH ** -0.5)
                if r0 < DIL * w:
                    pos = m * BM + r0 + lax.broadcasted_iota(jnp.int32, (n, 128), 0)
                    acc = jnp.where(pos >= DIL * w, acc, np.float32(-1e9))
                logits.append(acc)
            mx = functools.reduce(jnp.maximum, logits)
            e = [jnp.exp(l - mx) for l in logits]
            inv = 1.0 / functools.reduce(lambda a, b: a + b, e)
            pr = [t * inv for t in e]
            out = []
            for c in range(8):
                acc = None
                for w in range(WIN):
                    t = pr[w] * vb[c, pl.ds(HALO + r0 - DIL * w, n), :]
                    acc = t if acc is None else acc + t
                out.append(acc)
            return jnp.concatenate(out, axis=1)

        def block_step(m, carry):
            slot = m & 1

            @pl.when(m >= 2)
            def _():
                out_copy(m - 2, slot).wait()

            for c in range(8):
                kb[c, :HALO, :] = kb[c, BM:, :]
                vb[c, :HALO, :] = vb[c, BM:, :]
            project = lambda t: _dot(_unpack(_shifted(xn, m * BM, S - BM)[_rows(0, BM), :]),
                                     _unpack(wqt[:, t * D:(t + 1) * D]))
            for t, buf in ((2, vb), (1, kb)):
                val = project(t)
                for c in range(8):
                    buf[c, HALO:, :] = val[:, c * 128:(c + 1) * 128]
            q = project(0)
            for c in range(8):
                row0 = jnp.broadcast_to(vb[c, HALO:HALO + 1, :], (HALO, 128))
                vb[c, :HALO, :] = jnp.where(m == 0, row0, vb[c, :HALO, :])

            hv = _shifted(hs, m * BM, S - BM)
            h = _unpack(jnp.concatenate([hv[_rows(NC * S, BM), :F0]] + [hv[_rows(j * S, BM), :] for j in range(NC)],
                                        axis=1))
            seen, down = [], []
            for c in range(0, D, 128):
                acc = None
                for k in range(0, F, kd):
                    part = _dot(h[:, k:k + kd], wd_s[k:k + kd, c:c + 128])
                    acc = part if acc is None else acc + part
                    seen.append(acc)
                down.append(acc)
            down = jnp.concatenate(down, axis=1)
            pace = _pacer(seen, BM // att_rows, *att)
            o = jnp.concatenate([attend(m, q[r:r + att_rows], r, att_rows, pace())
                                 for r in range(0, BM, att_rows)], axis=0)
            proj = _dot(o.astype(BF16), _unpack(jnp.concatenate([wot[_rows(n * D, D), :] for n in range(2)], axis=1)))
            res = xs[pl.ds(pl.multiple_of(m * BM, BM), BM), :].astype(F32)
            outb.at[slot][...] = (res + proj * (down * jax.nn.sigmoid(down))).astype(BF16)
            out_copy(m, slot).start()
            return carry

        for c in range(8):
            kb[c, BM:, :] = jnp.zeros((HALO, 128), F32)
            vb[c, BM:, :] = jnp.zeros((HALO, 128), F32)
        with scope('p2'):
            lax.fori_loop(0, NB, scoped('p2_it', block_step), 0)
        with scope('tail'):
            out_copy(NB - 2, 0).wait()
            out_copy(NB - 1, 1).wait()

    def fn(A_x, A_wqkv, A_wo, B_x, B_w_gate, B_w_up, B_w_down):
        any_spec = pl.BlockSpec(memory_space=pl.ANY)
        out = pl.pallas_call(
            kernel,
            in_specs=[any_spec] * 6,
            out_specs=any_spec,
            out_shape=jax.ShapeDtypeStruct((S, D), BF16),
            scratch_shapes=[
                pltpu.VMEM((S, D), BF16),
                pltpu.VMEM((S // 2, D), U32),
                pltpu.VMEM(((NC + 1) * S // 2, FC), U32),
                pltpu.VMEM((D // 2, 3 * D), U32),
                pltpu.VMEM((D, 512), U32),
                pltpu.VMEM((2, D, FC), BF16),
                pltpu.VMEM((2, D, FC), BF16),
                pltpu.VMEM((F, D), BF16),
                pltpu.VMEM((D, 3 * D), BF16),
                pltpu.VMEM((2, D, 512), BF16),
                pltpu.VMEM((8, HALO + BM, 128), F32),
                pltpu.VMEM((8, HALO + BM, 128), F32),
                pltpu.VMEM((2, BM, D), BF16),
                pltpu.SemaphoreType.DMA((NB,)),
                pltpu.SemaphoreType.DMA((3, 2)),
                pltpu.SemaphoreType.DMA((3,)),
                pltpu.SemaphoreType.DMA((2,)),
            ],
            compiler_params=pltpu.CompilerParams(vmem_limit_bytes=100 * 2**20, flags=flags,
                                                 disable_bounds_checks=nobc, disable_semaphore_checks=nosc),
        )(A_x.reshape(S, D), A_wqkv, A_wo, B_w_gate, B_w_up, B_w_down)
        return out.reshape(1, S, D)

    return fn


@jax.jit
def pallas_recurrent_scan__sliding_local_dilated__geglu_ffn__prompt_kernel(
        A_x, A_wqkv, A_wo, B_x, B_w_gate, B_w_up, B_w_down):
    return make()(A_x, A_wqkv, A_wo, B_x, B_w_gate, B_w_up, B_w_down)
```

```python
import functools

import jax
import jax.numpy as jnp
import numpy as np
from jax import lax
import jax.experimental.pallas as pl
import jax.experimental.pallas.tpu as pltpu

S, D, F = 2048, 1024, 3584
HEAD, WINDOW, DILATION = 32, 8, 2
BM = 256
NB = S // BM
FC = 256
NC = F // FC
HALO = 16
OUT_CUTS = (0, 512, 768, 896, D)
F32, BF16, U32 = jnp.float32, jnp.bfloat16, jnp.uint32


def _pack(v):
    return pltpu.bitcast(v.astype(BF16), U32)


def _unpack(v):
    return pltpu.bitcast(v, BF16)


def _rows(start, n):
    return pl.ds(start // 2, n // 2)


def _shifted(ref, rows, limit):
    start = rows // 2 if isinstance(rows, int) else pl.multiple_of(rows >> 1, 8)
    return ref.at[pl.ds(start, ref.shape[0] - limit // 2)]


def _dot(a, b):
    return jnp.dot(a, b, preferred_element_type=F32)


def _geglu(g, u):
    c = np.sqrt(2.0 / np.pi)
    t = jnp.tanh(g * (np.float32(c) + np.float32(c * 0.044715) * (g * g)))
    return ((0.5 * g) * (1.0 + t)) * u


def _silu(d):
    return (0.5 * d) * (1.0 + jnp.tanh(0.5 * d))


def _unpaced():
    return lambda v: v


def _pacer(products, count, lo, hi):
    tiles = [(m, r, c) for m in products for c in range(0, m.shape[1], 128) for r in range(0, m.shape[0], 8)]
    calls = iter(range(count))

    def pace():
        k = int(np.floor((lo + (hi - lo) * next(calls) / count) * len(tiles)))
        if k < 0:
            return _unpaced()
        m, r, c = tiles[k]
        tile = m[r:r + 8, c:c + 128]

        def hold(v):
            never = jnp.tile(tile, (v.shape[0] // 8, v.shape[1] // 128)) > np.float32(np.inf)
            return jnp.where(never, jnp.zeros_like(v), v)
        return hold
    return pace


def _swap_tile_and_lane_bits(tiles):
    lane = lax.broadcasted_iota(jnp.int32, tiles[0].shape, 1)
    tiles = list(tiles)
    for t in range(3):
        s = 4 << t
        low = (lane & s) == 0
        for c in range(8):
            if not c & (1 << t):
                a, b = tiles[c], tiles[c | (1 << t)]
                tiles[c] = jnp.where(low, a, pltpu.roll(b, s, 1))
                tiles[c | (1 << t)] = jnp.where(low, pltpu.roll(a, 128 - s, 1), b)
    return tiles


def _kernel(x_hbm, wqkv_hbm, wo_hbm, wg_hbm, wu_hbm, wd_hbm, out_hbm,
            xs, xn, hs, wqkv, wo, wg, wu, wd, wqkv_raw, wo_raw, kb, vb,
            sem_x, sem_w, sem_once, sem_out, *out_bufs):

    def x_copy(m):
        rows = pl.ds(pl.multiple_of(m * BM, BM), BM)
        return pltpu.make_async_copy(x_hbm.at[rows], xs.at[rows], sem_x.at[m])

    def chunk_copies(j, k):
        cols = pl.ds(pl.multiple_of(j * FC, FC), FC)
        return (pltpu.make_async_copy(wg_hbm.at[:, cols], wg.at[j], sem_w.at[0, k]),
                pltpu.make_async_copy(wu_hbm.at[:, cols], wu.at[j], sem_w.at[1, k]))

    def wqkv_copy(i):
        rows = pl.ds(pl.multiple_of(i * 128, 128), 128)
        return pltpu.make_async_copy(wqkv_hbm.at[rows], wqkv_raw.at[rows], sem_w.at[2, i & 1])

    def wo_copy(n):
        return pltpu.make_async_copy(wo_hbm.at[:, n * 512:(n + 1) * 512], wo_raw.at[n], sem_once.at[n])

    def wd_copy():
        return pltpu.make_async_copy(wd_hbm, wd, sem_once.at[2])

    def out_copies(m, slot):
        rows = pl.ds(pl.multiple_of(m * BM, BM), BM)
        return [pltpu.make_async_copy(buf.at[slot], out_hbm.at[rows, c0:c1], sem_out.at[n, slot])
                for n, (buf, c0, c1) in enumerate(zip(out_bufs, OUT_CUTS[:-1], OUT_CUTS[1:]))]

    def layernorm(m, pace):
        src, dst = xs.at[pl.ds(pl.multiple_of(m * BM, BM), BM)], _shifted(xn, m * BM, S - BM)
        groups, lag, mean = range(0, BM, 16), 4, {}
        for n in range(len(groups) + lag):
            if n < len(groups):
                r = groups[n]
                x = src[r:r + 16, :].astype(F32)
                x = jnp.concatenate([pace()(x[:, :128]), x[:, 128:]], axis=1)
                mean[r] = jnp.broadcast_to(jnp.mean(x, axis=-1, keepdims=True), (16, 128))
            if n >= lag:
                r = groups[n - lag]
                xc = src[r:r + 16, :].astype(F32) - jnp.tile(pace()(mean[r]), (1, D // 128))
                dst[_rows(r, 16), :] = _pack(xc * lax.rsqrt(jnp.mean(xc * xc, axis=-1, keepdims=True) + 1e-5))

    def xn_block(m):
        return _unpack(_shifted(xn, m * BM, S - BM)[_rows(0, BM), :])

    def gate_up(t):
        j, m, products = t >> 3, t & 7, []
        for c in range(0, FC, 128):
            g = _dot(xn_block(m), wg.at[j][:, c:c + 128])
            u = _dot(xn_block(m), wu.at[j][:, c:c + 128])
            _shifted(hs, t * BM, NC * S - BM)[_rows(0, BM), c:c + 128] = _pack(_geglu(g, u))
            products += [g, u]
        return products

    def reorder_wqkv(i, t, r, hold):
        src = wqkv_raw.at[pl.ds(pl.multiple_of(i * 128, 128), 128)]
        tiles = [hold(pltpu.bitcast(src[r:r + 16, t * D + c * 128:t * D + (c + 1) * 128], U32)) for c in range(8)]
        _shifted(wqkv, i * 128, D - 128)[_rows(r, 16), t * D:(t + 1) * D] = jnp.concatenate(
            _swap_tile_and_lane_bits(tiles), axis=1)

    def reorder_wo(i, c2, d43, hold):
        n, r0 = i >> 2, pl.multiple_of((i & 3) * 32, 32)
        low = lax.broadcasted_iota(jnp.int32, (8, 512), 0) < 4
        src, dst = wo_raw.at[n, pl.ds(r0, D - 96)], _shifted(wo, n * D + r0, D + 96)
        t = [hold(src[pl.ds((4 * c2 + c) * 128 + d43 * 8, 8), :].astype(F32)) for c in range(4)]
        dst[_rows(2 * d43 * 128 + 16 * c2, 16), :] = _pack(jnp.concatenate(
            [jnp.where(low, t[c], pltpu.roll(t[c + 1], 4, 0)) for c in (0, 2)], axis=0))
        dst[_rows((2 * d43 + 1) * 128 + 16 * c2, 16), :] = _pack(jnp.concatenate(
            [jnp.where(low, pltpu.roll(t[c], 4, 0), t[c + 1]) for c in (0, 2)], axis=0))

    gate0, up0 = chunk_copies(0, 0)
    x_copy(0).start()
    x_copy(1).start()

    def first_rows(m, carry):
        x_copy(m).wait()
        pl.when(m == 0)(gate0.start)

        @pl.when(m == 1)
        def _():
            up0.start()
            x_copy(2).start()

        layernorm(m, _unpaced)
        return carry

    lax.fori_loop(0, 2, first_rows, 0)
    gate0.wait()
    x_copy(3).start()
    g = _dot(_unpack(xn[_rows(0, 2 * BM), :]), wg[0])
    up0.wait()
    x_copy(2).wait()
    x_copy(4).start()
    u = _dot(_unpack(xn[_rows(0, 2 * BM), :]), wu[0])
    hs[_rows(0, 2 * BM), :] = _pack(_geglu(g, u))
    layernorm(2, _pacer([u], 32, -0.1, 0.9))
    for blocks, prefetch in (
            ((2, 3), lambda: (x_copy(5), x_copy(6), x_copy(7))),
            ((4, 5, 6, 7), lambda: (*chunk_copies(1, 0), *chunk_copies(2, 1), wqkv_copy(0), wo_copy(0)))):
        for m in blocks:
            if m + 1 < NB:
                x_copy(m + 1).wait()
        for copy in prefetch():
            copy.start()
        for m in blocks:
            products = gate_up(m)
            if m + 1 < NB:
                layernorm(m + 1, _pacer(products, 32, -0.1 if m == blocks[0] else 0.0, 0.9))
    wo_copy(0).wait()

    def ffn_step(i, carry):
        wqkv_copy(i).wait()
        for k in range(2):
            @pl.when(2 * i + 1 + k < NC)
            def _():
                for copy in chunk_copies(2 * i + 1 + k, k):
                    copy.wait()

        @pl.when(i == 4)
        def _():
            wo_copy(1).wait()

        for k in range(2):
            @pl.when(2 * i + 3 + k < NC)
            def _():
                for copy in chunk_copies(2 * i + 3 + k, k):
                    copy.start()

        @pl.when(i + 1 < NB)
        def _():
            wqkv_copy(i + 1).start()

        @pl.when(i == 3)
        def _():
            wo_copy(1).start()

        @pl.when(i == 6)
        def _():
            wd_copy().start()

        products = [p for t in range(NC - 1) for p in gate_up(NB + (NC - 1) * i + t)]
        pace = _pacer(products, 32, 0.0, 0.9)
        for r in range(8):
            for t in range(3):
                reorder_wqkv(i, t, r * 16, pace())
            reorder_wo(i, r // 4, r % 4, pace())
        return carry

    lax.fori_loop(0, NB, ffn_step, 0)
    wd_copy().wait()

    def attend(m, q, r0, hold):
        lane = lax.broadcasted_iota(jnp.int32, (8, 128), 1)
        window = [pl.ds(HALO + r0 - DILATION * w, 8) for w in range(WINDOW)]
        total = functools.partial(functools.reduce, jnp.add)
        q = [hold(q[:, c * 128:(c + 1) * 128]) for c in range(8)]
        logits = []
        for w in range(WINDOW):
            acc = total([q[c] * kb[c, window[w], :] for c in range(8)])
            for s in (1, 2):
                acc = acc + jnp.take_along_axis(acc, lane ^ s, axis=1)
            acc = acc * np.float32(HEAD ** -0.5)
            if r0 < DILATION * w:
                pos = m * BM + r0 + lax.broadcasted_iota(jnp.int32, (8, 128), 0)
                acc = jnp.where(pos >= DILATION * w, acc, np.float32(-1e9))
            logits.append(acc)
        top = functools.reduce(jnp.maximum, logits)
        e = [jnp.exp(l - top) for l in logits]
        inv = 1.0 / total(e)
        p = [t * inv for t in e]
        return jnp.concatenate(
            [total([p[w] * vb[c, window[w], :] for w in range(WINDOW)]) for c in range(8)], axis=1)

    def block_step(m, carry):
        slot = m & 1

        @pl.when(m >= 2)
        def _():
            for copy in out_copies(m - 2, slot):
                copy.wait()

        for c in range(8):
            kb[c, :HALO, :] = kb[c, BM:, :]
            vb[c, :HALO, :] = vb[c, BM:, :]
        project = lambda t: _dot(xn_block(m), _unpack(wqkv[:, t * D:(t + 1) * D]))
        for t, buf in ((2, vb), (1, kb)):
            val = project(t)
            for c in range(8):
                buf[c, HALO:, :] = val[:, c * 128:(c + 1) * 128]
        q = project(0)
        for c in range(8):
            first = jnp.broadcast_to(vb[c, HALO:HALO + 1, :], (HALO, 128))
            vb[c, :HALO, :] = jnp.where(m == 0, first, vb[c, :HALO, :])

        h_rows = _shifted(hs, m * BM, S - BM)
        h = _unpack(jnp.concatenate([h_rows[_rows(j * S, BM), :] for j in range(NC)], axis=1))
        partial, down = [], []
        for c in range(0, D, 128):
            for k in range(0, F, 512):
                part = _dot(h[:, k:k + 512], wd[k:k + 512, c:c + 128])
                partial.append(part if k == 0 else partial[-1] + part)
            down.append(partial[-1])

        pace = _pacer(partial, BM // 8, 0.1, 0.94)
        o = jnp.concatenate([attend(m, q[r:r + 8], r, pace()) for r in range(0, BM, 8)], axis=0)
        s = _dot(o.astype(BF16), _unpack(jnp.concatenate([wo[_rows(n * D, D), :] for n in range(2)], axis=1)))
        x = xs[pl.ds(pl.multiple_of(m * BM, BM), BM), :].astype(F32)
        out = (x + s * _silu(jnp.concatenate(down, axis=1))).astype(BF16)
        for buf, c0, c1, copy in zip(out_bufs, OUT_CUTS[:-1], OUT_CUTS[1:], out_copies(m, slot)):
            buf.at[slot][...] = out[:, c0:c1]
            copy.start()
        return carry

    for c in range(8):
        kb[c, BM:, :] = jnp.zeros((HALO, 128), F32)
        vb[c, BM:, :] = jnp.zeros((HALO, 128), F32)
    lax.fori_loop(0, NB, block_step, 0)
    for copy in out_copies(NB - 2, 0) + out_copies(NB - 1, 1):
        copy.wait()


@jax.jit
def pallas_recurrent_scan__sliding_local_dilated__geglu_ffn__prompt_kernel(
    A_x: jax.Array,
    A_wqkv: jax.Array,
    A_wo: jax.Array,
    B_x: jax.Array,
    B_w_gate: jax.Array,
    B_w_up: jax.Array,
    B_w_down: jax.Array,
):
    del B_x
    hbm = pl.BlockSpec(memory_space=pl.ANY)
    out = pl.pallas_call(
        _kernel,
        in_specs=[hbm] * 6,
        out_specs=hbm,
        out_shape=jax.ShapeDtypeStruct((S, D), BF16),
        scratch_shapes=[
            pltpu.VMEM((S, D), BF16),
            pltpu.VMEM((S // 2, D), U32),
            pltpu.VMEM((NC * S // 2, FC), U32),
            pltpu.VMEM((D // 2, 3 * D), U32),
            pltpu.VMEM((D, 512), U32),
            pltpu.VMEM((NC, D, FC), BF16),
            pltpu.VMEM((NC, D, FC), BF16),
            pltpu.VMEM((F, D), BF16),
            pltpu.VMEM((D, 3 * D), BF16),
            pltpu.VMEM((2, D, 512), BF16),
            pltpu.VMEM((8, HALO + BM, 128), F32),
            pltpu.VMEM((8, HALO + BM, 128), F32),
            pltpu.SemaphoreType.DMA((NB,)),
            pltpu.SemaphoreType.DMA((3, 2)),
            pltpu.SemaphoreType.DMA((3,)),
            pltpu.SemaphoreType.DMA((len(OUT_CUTS) - 1, 2)),
            *[pltpu.VMEM((2, BM, c1 - c0), BF16) for c0, c1 in zip(OUT_CUTS[:-1], OUT_CUTS[1:])],
        ],
        compiler_params=pltpu.CompilerParams(
            vmem_limit_bytes=100 * 2**20,
            disable_bounds_checks=True,
            flags={"XLA_TPU_EVENLY_DISTRIBUTE_CRITICAL_NODES": True},
        ),
    )(A_x.reshape(S, D), A_wqkv, A_wo, B_w_gate, B_w_up, B_w_down)
    return out.reshape(1, S, D)
```
